```python
import jax
import jax.numpy as jnp

def _softmax(x, axis=-1):
    return jax.nn.softmax(x, axis=axis)

def _gelu(x):
    return jax.nn.gelu(x, approximate=True)

def _silu(x):
    return jax.nn.silu(x)

def _sigmoid(x):
    return jax.nn.sigmoid(x)

def _layernorm(x, axis=-1, eps=1e-05):
    m = jnp.mean(x, axis=axis, keepdims=True)
    v = jnp.var(x, axis=axis, keepdims=True)
    return (x - m) / jnp.sqrt(v + eps)

def _scatter_add(tgt, idx, src, axis=0):
    return tgt.at[idx].add(src)

def _segment_sum(src, seg, n):
    return jax.ops.segment_sum(src, seg, n)

class _Rng:

    def __init__(self, key):
        self._k = key

    def _next(self):
        self._k, sub = jax.random.split(self._k)
        return sub

    def normal(self, shape):
        return jax.random.normal(self._next(), shape, dtype=jnp.bfloat16)

    def randint(self, lo, hi, shape):
        return jax.random.randint(self._next(), shape, lo, hi, dtype=jnp.int32)

    def uniform(self, shape, lo=0.0, hi=1.0):
        return jax.random.uniform(self._next(), shape, jnp.bfloat16, lo, hi)

    def permutation(self, n):
        return jax.random.permutation(self._next(), n)
kernel_name = 'adaLN_cond__ssm_conv_h3__glu_gated_reglu__prompt'

def setup_inputs():
    _rng = _Rng(jax.random.key(int.from_bytes(__import__("os").urandom(4), "little")))
    _w = lambda a: (lambda t: t.astype(jnp.bfloat16) if jnp.issubdtype(t.dtype, jnp.floating) else t)(jnp.asarray(a))

    def _A_setup():
        B, S, D = (1, 2048, 640)
        ks = 4
        return {'q': _w((lambda *s: _rng.normal(s) * 0.05)(B, S, D)), 'k': _w((lambda *s: _rng.normal(s) * 0.05)(B, S, D)), 'v': _w((lambda *s: _rng.normal(s) * 0.05)(B, S, D)), 'shift_k': _w((lambda *s: _rng.normal(s) * 0.05)(D, ks) * 0.5), 'ssm_k': _w((lambda *s: _rng.normal(s) * 0.05)(D, S) * (1.0 / S ** 0.5)), 'ssm_D': _w((lambda *s: _rng.normal(s) * 0.05)(D))}
    _A_in = _A_setup()

    def _B_setup():
        B, S, D, F = (1, 2048, 640, 1536)
        return {'x': _w((lambda *s: _rng.normal(s) * 0.05)(B, S, D)), 'W_gate': _w((lambda *s: _rng.normal(s) * 0.05)(D, F) * (2.0 / D) ** 0.5), 'W_up': _w((lambda *s: _rng.normal(s) * 0.05)(D, F) * (2.0 / D) ** 0.5), 'W_down': _w((lambda *s: _rng.normal(s) * 0.05)(F, D) * (1.0 / F) ** 0.5)}
    _B_in = _B_setup()
    return {'A_q': _A_in['q'], 'A_k': _A_in['k'], 'A_v': _A_in['v'], 'A_shift_k': _A_in['shift_k'], 'A_ssm_k': _A_in['ssm_k'], 'A_ssm_D': _A_in['ssm_D'], 'B_x': _B_in['x'], 'B_W_gate': _B_in['W_gate'], 'B_W_up': _B_in['W_up'], 'B_W_down': _B_in['W_down'], 'c': _w((lambda *s: _rng.normal(s) * 0.05)(1, 640)), 'w_mod': _w((lambda *s: _rng.normal(s) * 0.05)(640, 6 * 640) * 640 ** (-0.5))}

def reference(A_q, A_k, A_v, A_shift_k, A_ssm_k, A_ssm_D, B_x, B_W_gate, B_W_up, B_W_down, c, w_mod):

    def _A_ref(q, k, v, shift_k, ssm_k, ssm_D):
        B, S, D = q.shape
        ks = shift_k.shape[-1]
        k_pad = jnp.pad(k, ((0, 0), (ks - 1, 0), (0, 0)))
        k_shift = jnp.zeros_like(k)
        for t in range(ks):
            k_shift = k_shift + k_pad[:, t:t + S, :] * shift_k[:, ks - 1 - t][None, None, :]
        kv = k_shift * v
        L = 2 * S
        kv_pad = jnp.pad(kv, ((0, 0), (0, S), (0, 0)))
        kf_pad = jnp.pad(ssm_k, ((0, 0), (0, S)))
        kv_f = (lambda x, axes=(-2, -1): jnp.fft.rfft2(x.astype(jnp.float32), axes=axes))(kv_pad[:, None, :, :], axes=(1, 2))
        kf_f = (lambda x, axes=(-2, -1): jnp.fft.rfft2(x.astype(jnp.float32), axes=axes))(kf_pad[:, None, :], axes=(1, 2))
        kf_f = (lambda x, *d: x.transpose(*d))(kf_f, 1, 2, 0)
        y_f = kv_f * kf_f[None, :, :, :]
        y = (lambda x, s, axes=(-2, -1): jnp.fft.irfft2(x, s=s, axes=axes).astype(jnp.bfloat16))(y_f, (1, L), axes=(1, 2))[:, 0, :S, :]
        y = y + kv * ssm_D[None, None, :]
        return q * y

    def _B_ref(x, W_gate, W_up, W_down):
        gate = jnp.einsum('bsd,df->bsf', x, W_gate)
        up = jnp.einsum('bsd,df->bsf', x, W_up)
        gate = gate * (lambda x, dt: x.astype(dt))(gate > 0, gate.dtype)
        h = gate * up
        return jnp.einsum('bsf,fd->bsd', h, W_down)
    x = A_q
    mod = (_silu(c) @ w_mod).reshape(c.shape[0], 6, 1, -1)
    sa, ca, ga, sb, cb, gb = (mod[:, 0].copy(), mod[:, 1].copy(), mod[:, 2].copy(), mod[:, 3].copy(), mod[:, 4].copy(), mod[:, 5].copy())
    h = _layernorm(x, axis=-1) * (1 + ca) + sa
    x = x + ga * _A_ref(h, A_k, A_v, A_shift_k, A_ssm_k, A_ssm_D)
    h = _layernorm(x, axis=-1) * (1 + cb) + sb
    x = x + gb * _B_ref(h, B_W_gate, B_W_up, B_W_down)
    return x
```

```python
import numpy as np
import jax
import jax.numpy as jnp
from jax import lax
import jax.experimental.pallas as pl
import jax.experimental.pallas.tpu as pltpu

S, D, F = 2048, 640, 1536
L = 512
NC = S // L
NT = D // 128
MB = 256
NB = S // MB
PR = 16
KD = 4
FU = 4
IU = 4
CU = 4
GW = {0: 2, 4: 4, 8: 6}
DW = {0: 2, 2: 5}
LATE_AT = 0
PAD = 8
MOD_A, MOD_B = (0, 1), (2, 3)
Q1W = 4
IA, IB, PA = 0.0, 0.18, 0.24
SCOPES = False
f32, bf16, u32 = jnp.float32, jnp.bfloat16, jnp.uint32


def _dft_consts():
    k = np.arange(128, dtype=np.float64)[:, None]
    m = np.arange(128, dtype=np.float64)[None, :]
    perm = np.arange(256).reshape(2, 16, 8).transpose(1, 0, 2).reshape(-1)
    Fm, Fi = [], []
    for r in range(4):
        ph = 2.0 * np.pi * (k + 0.25) / L * (4 * m + r)
        f = np.concatenate([np.cos(ph), np.sin(ph)], axis=0)[perm]
        Fm.append(f)
        Fi.append(f.T / L)
    return np.stack(Fm), np.stack(Fi)


def _ln(x):
    m = jnp.sum(x, axis=-1, keepdims=True) * (1.0 / D)
    xc = x - m
    v = jnp.sum(xc * xc, axis=-1, keepdims=True) * (1.0 / D)
    return xc * lax.rsqrt(v + 1e-5)


def _lo(w):
    return lax.bitcast_convert_type(w << 16, f32)


def _hi(w):
    return lax.bitcast_convert_type(w & jnp.uint32(0xFFFF0000), f32)


def _bfly_fwd(a):
    (a0r, a0i), (a1r, a1i), (a2r, a2i), (a3r, a3i) = a
    t0r, t0i, t1r, t1i = a0r + a2r, a0i + a2i, a0r - a2r, a0i - a2i
    t2r, t2i, t3r, t3i = a1r + a3r, a1i + a3i, a1r - a3r, a1i - a3i
    return [(t0r + t2r, t0i + t2i), (t1r - t3i, t1i + t3r), (t0r - t2r, t0i - t2i), (t1r + t3i, t1i - t3r)]


def _bfly_inv(q):
    (q0r, q0i), (q1r, q1i), (q2r, q2i), (q3r, q3i) = q
    u0r, u0i, u1r, u1i = q0r + q2r, q0i + q2i, q0r - q2r, q0i - q2i
    u2r, u2i, u3r, u3i = q1r + q3r, q1i + q3i, q1r - q3r, q1i - q3i
    return [(u0r + u2r, u0i + u2i), (u1r + u3i, u1i - u3r), (u0r - u2r, u0i - u2i), (u1r - u3i, u1i + u3r)]


def interleave(main, nmain, sides):
    done = [0] * len(sides)
    i = 0
    for _ in main:
        i += 1
        f = i / nmain
        for s, (g, n, a, b) in enumerate(sides):
            want = min(n, max(0, int(np.ceil((f - a) / (b - a) * n - 1e-9))))
            while done[s] < want:
                next(g)
                done[s] += 1
    for s, (g, n, a, b) in enumerate(sides):
        while done[s] < n:
            next(g)
            done[s] += 1
        for _ in g:
            pass


class _NoScope:
    def __init__(self, name): pass
    def __enter__(self): return self
    def __exit__(self, *a): return False


def kernel(q_hbm, k_hbm, v_hbm, skt_ref, ssmk_hbm, ssmd_ref, wg_hbm, wu_hbm, wd_hbm, c_ref, wmod_hbm,
           F_hbm, Fi_hbm, o_hbm, F_ref, Fi_ref,
           k_s, v_s, ssmk_s, kt_s, xs, gs, qs, y_s, q_s, wg_s, wu_s, wd_s, wmod_s, mod_s,
           x1_s, h2_s, hh_s, o_s, sems, osems):
    scope = jax.named_scope if SCOPES else _NoScope

    def conv_copies(c):
        c0 = c * 128 if isinstance(c, int) else pl.multiple_of(c * 128, 128)
        return [pltpu.make_async_copy(ssmk_hbm.at[pl.ds(c0, 128), :], ssmk_s.at[c], sems.at[c]),
                pltpu.make_async_copy(k_hbm.at[:, pl.ds(c0, 128)], k_s.at[c, pl.ds(16, S), :], sems.at[NT + c]),
                pltpu.make_async_copy(v_hbm.at[:, pl.ds(c0, 128)], v_s.at[c], sems.at[2 * NT + c])]

    nsem = [3 * NT + NB]

    def cp(src, dst):
        nsem[0] += 1
        return pltpu.make_async_copy(src, dst, sems.at[nsem[0] - 1])
    F_cp = cp(F_hbm, F_ref)
    Fi_cp = cp(Fi_hbm, Fi_ref)
    wmod_cps = [cp(wmod_hbm.at[i * 128:(i + 1) * 128, :], wmod_s.at[i * 128:(i + 1) * 128, :]) for i in range(NT)]
    WP = 256
    wg_cps = [cp(wg_hbm.at[:, n * WP:(n + 1) * WP], wg_s.at[:, n * WP:(n + 1) * WP]) for n in range(F // WP)]
    wu_cps = [cp(wu_hbm.at[:, n * WP:(n + 1) * WP], wu_s.at[:, n * WP:(n + 1) * WP]) for n in range(F // WP)]
    wd_cps = [cp(wd_hbm.at[:, n * 128:(n + 1) * 128], wd_s.at[:, n * 128:(n + 1) * 128]) for n in range(NT)]

    def q_copy(b):
        r0 = b * MB if isinstance(b, int) else pl.multiple_of(b * MB, MB)
        return pltpu.make_async_copy(q_hbm.at[pl.ds(r0, MB), :], q_s.at[pl.ds(r0, MB), :], sems.at[3 * NT + b])

    cps0 = conv_copies(0)
    cps0[0].start()
    F_cp.start()
    cps0[1].start()
    cps0[2].start()
    Fi_cp.start()
    for c in range(1, NT):
        for d in conv_copies(c):
            d.start()

    def start_late():
        for d in wmod_cps:
            d.start()
        q_copy(0).start()
        for n in range(F // WP):
            wg_cps[n].start()
            wu_cps[n].start()
            if n == 2:
                q_copy(1).start()
        for d in wd_cps:
            d.start()
        for b in range(2, NB):
            q_copy(b).start()

    for c in range(NT):
        k_s[c, 0:16, :] = jnp.zeros((16, 128), bf16)

    def T_tile(c, t):
        t0 = t * 128 if isinstance(t, int) else pl.multiple_of(t * 128, 128)
        kt_s[pl.ds(t0, 128), :] = ssmk_s[c, :, pl.ds(t0, 128)].T

    def phases(wref, off):
        a = wref[pl.ds(off, 128, stride=2), :]
        b = wref[pl.ds(off + 1, 128, stride=2), :]
        return [_lo(a), _hi(a), _lo(b), _hi(b)]

    def spectrum(parts, dst, j, first, extra=None):
        for g in range(16):
            a = [(parts[r][16 * g:16 * g + 8], parts[r][16 * g + 8:16 * g + 16]) for r in range(4)]
            if extra is not None:
                a[0] = (a[0][0] + extra, a[0][1])
            for q, (re, im) in enumerate(_bfly_fwd(a)):
                if first:
                    trip = (re + im, re, im)
                else:
                    trip = (re, im - re, re + im)
                for u in range(3):
                    dst[j, q, u, 8 * g:8 * g + 8, :] = trip[u]

    def F_chunk(c, j):
        c0 = pl.multiple_of(c * 128, 128) if not isinstance(c, int) else c * 128
        w0 = pl.multiple_of(j * (L // 2), L // 2)
        kk = phases(kt_s.bitcast(u32).at[pl.ds(w0, L // 2), :], 0)
        kparts = [jnp.dot(F_ref[r], kk[r].astype(bf16), preferred_element_type=f32) for r in range(4)]
        w = skt_ref[:, pl.ds(c0, 128)].astype(f32)
        kw = k_s.bitcast(u32).at[c, pl.ds(w0, L // 2 + 8), :]
        vw = v_s.bitcast(u32).at[c, pl.ds(w0, L // 2), :]
        kc = phases(kw, 8)
        kp = phases(kw, 6)
        vv = phases(vw, 0)
        taps = [[kc[0], kp[3], kp[2], kp[1]], [kc[1], kc[0], kp[3], kp[2]],
                [kc[2], kc[1], kc[0], kp[3]], [kc[3], kc[2], kc[1], kc[0]]]
        parts = []
        for r in range(4):
            ks = taps[r][0] * w[0:1] + taps[r][1] * w[1:2] + taps[r][2] * w[2:3] + taps[r][3] * w[3:4]
            kv = (ks * vv[r]).astype(bf16)
            parts.append(jnp.dot(F_ref[r], kv, preferred_element_type=f32))
        sd = jnp.where(j == 0, ssmd_ref[:, pl.ds(c0, 128)].astype(f32), 0.0)
        spectrum(kparts, gs, j, False, extra=sd)
        spectrum(parts, xs, j, True)

    def C_pos(p):
        r0 = pl.multiple_of(p * 8, 8)
        for q in range(4):
            X = [tuple(xs[j, q, u, pl.ds(r0, 8), :] for u in range(3)) for j in range(NC)]
            G = [tuple(gs[m, q, u, pl.ds(r0, 8), :] for u in range(3)) for m in range(NC)]
            prev = None
            for i in range(NC):
                acc = None
                for j in range(i + 1):
                    s, xr, xi = X[j]
                    gr, d, t = G[i - j]
                    q3 = (gr * s, xr * d, xi * t)
                    acc = q3 if acc is None else (acc[0] + q3[0], acc[1] + q3[1], acc[2] + q3[2])
                pr, pi = acc[0] - acc[2], acc[0] + acc[1]
                qr, qi = (pr, pi) if prev is None else (pr + prev[1], pi - prev[0])
                prev = (pr, pi)
                qs[i, q, 0, pl.ds(r0, 8), :] = qr
                qs[i, q, 1, pl.ds(r0, 8), :] = qi

    def I_chunk(c, j):
        r0 = j * L if isinstance(j, int) else pl.multiple_of(j * L, L)
        yv = y_s.at[c, pl.ds(r0, L), :]
        rows = [[] for _ in range(4)]
        for g in range(16):
            Q = [(qs[j, q, 0, 8 * g:8 * g + 8, :], qs[j, q, 1, 8 * g:8 * g + 8, :]) for q in range(4)]
            for r, (br, bi) in enumerate(_bfly_inv(Q)):
                rows[r].append(jnp.concatenate([br, bi], axis=0).astype(bf16))
        for r in range(4):
            yv[pl.ds(r, 128, stride=4), :] = jnp.dot(Fi_ref[r], jnp.concatenate(rows[r], axis=0),
                                                     preferred_element_type=f32)

    def loop(n, fn):
        def body(i, carry):
            fn(i)
            return carry
        lax.fori_loop(0, n, body, 0)

    def C_iter(po):
        for u in range(CU):
            C_pos(po * CU + u)

    def mod_part(i):
        wmod_cps[i].wait()
        cf = c_ref[:, i * 128:(i + 1) * 128].astype(f32)
        sc = (cf * jax.nn.sigmoid(cf)).astype(bf16)
        acc = jnp.dot(sc, wmod_s[i * 128:(i + 1) * 128, :], preferred_element_type=f32)
        if i > 0:
            acc = acc + mod_s[...]
        if i == NT - 1:
            acc = acc.astype(bf16).astype(f32)
        mod_s[...] = acc

    with scope("wait0"):
        cps0[0].wait()
        for t in range(16):
            T_tile(0, t)
        F_cp.wait()

    def tile_body(c, last=False):
        cps = conv_copies(c)
        with scope("wkv"):
            cps[1].wait()
            cps[2].wait()
        if not last:
            pl.when(c == LATE_AT)(start_late)
        else:
            with scope("mod"):
                for i in MOD_A:
                    mod_part(i)
        with scope("F"):
            def f_body(jo):
                for u in range(FU):
                    F_chunk(c, jo * FU + u)
            loop(NC // FU, f_body)
        with scope("C"):
            if last:
                for i in MOD_B:
                    mod_part(i)
            loop(16 // CU, C_iter)
        if last:
            with scope("mod"):
                for i in range(MOD_B[-1] + 1, NT):
                    mod_part(i)
            return
        with scope("w"):
            pl.when(c == 0)(lambda: Fi_cp.wait())
            conv_copies(c + 1)[0].wait()
        with scope("I"):
            def i_body(jo):
                for u in range(IU):
                    I_chunk(c, jo * IU + u)
                    for t in range(4):
                        T_tile(c + 1, (jo * IU + u) * 4 + t)
            loop(NC // IU, i_body)
    with scope("conv"):
        loop(NT - 1, tile_body)
        tile_body(NT - 1, last=True)

    def pre_gen(b, slot):
        for p in range(MB // PR):
            r0 = b * MB + p * PR
            if not isinstance(r0, int):
                r0 = pl.multiple_of(r0, PR)
            sa = mod_s[:, 0 * D:1 * D]
            ca = mod_s[:, 1 * D:2 * D]
            ga = mod_s[:, 2 * D:3 * D]
            sb = mod_s[:, 3 * D:4 * D]
            cb = mod_s[:, 4 * D:5 * D]
            x = q_s[pl.ds(r0, PR), :].astype(f32)
            y = jnp.concatenate([y_s[c, pl.ds(r0, PR), :] for c in range(NT)], axis=1)
            h = _ln(x) * (1.0 + ca) + sa
            x1 = (x + ga * (h * y)).astype(bf16)
            x1_s[slot, p * PR:(p + 1) * PR, :] = x1
            x1 = x1.astype(f32)
            h2_s[slot, p * PR:(p + 1) * PR, :] = (_ln(x1) * (1.0 + cb) + sb).astype(bf16)
            yield

    def mlp_gen(slot, first=False):
        for n in range(F // 128):
            cs = slice(n * 128, (n + 1) * 128)
            a = h2_s[slot]
            if first and n in GW:
                with scope("wgw"):
                    for i in range(n * 128 // WP, GW[n]):
                        wg_cps[i].wait()
                        wu_cps[i].wait()
                    if n == Q1W:
                        q_copy(1).wait()
            g = jnp.dot(a, wg_s[:, cs], preferred_element_type=f32)
            yield
            u = jnp.dot(a, wu_s[:, cs], preferred_element_type=f32)
            hh_s[:, cs] = (jnp.maximum(g, 0.0) * u).astype(bf16)
            yield
        for n in range(NT):
            cs = slice(n * 128, (n + 1) * 128)
            acc = None
            if first and n in DW:
                with scope("wdw"):
                    for i in range(n, DW[n]):
                        wd_cps[i].wait()
            for kk in range(0, F // 128, KD):
                ks = slice(kk * 128, (kk + KD) * 128)
                d1 = jnp.dot(hh_s[:, ks], wd_s[ks, cs], preferred_element_type=f32)
                acc = d1 if acc is None else acc + d1
                if kk + KD >= F // 128:
                    gb = mod_s[:, 5 * D + n * 128:5 * D + (n + 1) * 128]
                    o_s[slot, :, cs] = (x1_s[slot, :, cs].astype(f32) + gb * acc).astype(bf16)
                yield
    NM = 2 * (F // 128) + NT * (F // 128 // KD)

    def out_copy(b, slot):
        return pltpu.make_async_copy(o_s.at[slot], o_hbm.at[pl.ds(pl.multiple_of(b * MB, MB), MB), :], osems.at[slot])

    def i_gen(c, chunks):
        for j in chunks:
            I_chunk(c, j)
            yield

    with scope("pre0"):
        I_chunk(NT - 1, 0)
        q_copy(0).wait()
        for _ in pre_gen(0, 0):
            pass
    with scope("blk0"):
        interleave(mlp_gen(0, first=True), NM, [(i_gen(NT - 1, range(1, NC)), NC - 1, IA, IB),
                                                (pre_gen(1, 1), MB // PR, PA, 0.95)])
        out_copy(0, 0).start()

    with scope("main"):
        def main_body(b, carry):
            slot = b % 2
            @pl.when(b >= 2)
            def _():
                out_copy(b - 2, slot).wait()
            q_copy(b + 1).wait()
            interleave(mlp_gen(slot), NM, [(pre_gen(b + 1, 1 - slot), MB // PR, 0.0, 0.95)])
            out_copy(b, slot).start()
            return carry
        lax.fori_loop(1, NB - 1, main_body, 0)
    with scope("last"):
        out_copy(NB - 3, (NB - 3) % 2).wait()
        for _ in mlp_gen((NB - 1) % 2):
            pass
        out_copy(NB - 1, (NB - 1) % 2).start()
    with scope("tail"):
        out_copy(NB - 2, (NB - 2) % 2).wait()
        out_copy(NB - 1, (NB - 1) % 2).wait()


@jax.jit
def pallas_adaLN_cond__ssm_conv_h3__glu_gated_reglu__prompt_kernel(
        A_q, A_k, A_v, A_shift_k, A_ssm_k, A_ssm_D, B_x, B_W_gate, B_W_up, B_W_down, c, w_mod):
    Fm, Fi = _dft_consts()
    Fm = jnp.asarray(Fm.astype(np.float32)).astype(bf16)
    Fi = jnp.asarray(Fi.astype(np.float32)).astype(bf16)
    hbm = pl.BlockSpec(memory_space=pl.ANY)
    vm = pl.BlockSpec(memory_space=pltpu.VMEM)
    out = pl.pallas_call(
        kernel,
        out_shape=jax.ShapeDtypeStruct((S, D), A_q.dtype),
        in_specs=[hbm, hbm, hbm, vm, hbm, vm, hbm, hbm, hbm, vm, hbm, hbm, hbm],
        out_specs=hbm,
        scratch_shapes=[
            pltpu.VMEM((4, 256, 128), bf16),
            pltpu.VMEM((4, 128, 256), bf16),
            pltpu.VMEM((NT, S + 16, 128), bf16),
            pltpu.VMEM((NT, S, 128), bf16),
            pltpu.VMEM((NT, 128, S), bf16),
            pltpu.VMEM((S, 128), bf16),
            pltpu.VMEM((NC, 4, 3, 128 + PAD, 128), f32),
            pltpu.VMEM((NC, 4, 3, 128 + PAD, 128), f32),
            pltpu.VMEM((NC, 4, 2, 128 + PAD, 128), f32),
            pltpu.VMEM((NT, S + PAD, 128), f32),
            pltpu.VMEM((S, D), bf16),
            pltpu.VMEM((D, F), bf16),
            pltpu.VMEM((D, F), bf16),
            pltpu.VMEM((F, D), bf16),
            pltpu.VMEM((D, 6 * D), bf16),
            pltpu.VMEM((1, 6 * D), f32),
            pltpu.VMEM((2, MB, D), bf16),
            pltpu.VMEM((2, MB, D), bf16),
            pltpu.VMEM((MB, F), bf16),
            pltpu.VMEM((2, MB, D), bf16),
            pltpu.SemaphoreType.DMA((3 * NT + NB + 2 + 2 * (F // 256) + 2 * NT,)),
            pltpu.SemaphoreType.DMA((2,)),
        ],
        compiler_params=pltpu.CompilerParams(vmem_limit_bytes=120 * 1024 * 1024),
    )(A_q.reshape(S, D), A_k.reshape(S, D), A_v.reshape(S, D), A_shift_k.T, A_ssm_k, A_ssm_D.reshape(1, D),
      B_W_gate, B_W_up, B_W_down, c, w_mod, Fm, Fi)
    return out.reshape(A_q.shape)
```

```python
import numpy as np
import jax
import jax.numpy as jnp
from jax import lax
import jax.experimental.pallas as pl
import jax.experimental.pallas.tpu as pltpu

S, D, F = 2048, 640, 1536
L = 512
NC = S // L
NT = D // 128
MB = 256
NB = S // MB
PR = 16
KD = 4
FU = 4
IU = 4
CU = 4
GW = {0: 2, 4: 4, 8: 6}
DW = {0: 2, 2: 5}
LATE_AT = 0
PAD = 8
MOD_A, MOD_B = (0, 1), (2, 3)
Q1W = 4
IA, IB, PA = 0.0, 0.18, 0.24
SCOPES = False
f32, bf16, u32 = jnp.float32, jnp.bfloat16, jnp.uint32


def _dft_consts():
    k = np.arange(128, dtype=np.float64)[:, None]
    m = np.arange(128, dtype=np.float64)[None, :]
    perm = np.arange(256).reshape(2, 16, 8).transpose(1, 0, 2).reshape(-1)
    Fm, Fi = [], []
    for r in range(4):
        ph = 2.0 * np.pi * (k + 0.25) / L * (4 * m + r)
        f = np.concatenate([np.cos(ph), np.sin(ph)], axis=0)[perm]
        Fm.append(f)
        Fi.append(f.T / L)
    return np.stack(Fm), np.stack(Fi)


def _ln(x):
    m = jnp.sum(x, axis=-1, keepdims=True) * (1.0 / D)
    xc = x - m
    v = jnp.sum(xc * xc, axis=-1, keepdims=True) * (1.0 / D)
    return xc * lax.rsqrt(v + 1e-5)


def _lo(w):
    return lax.bitcast_convert_type(w << 16, f32)


def _hi(w):
    return lax.bitcast_convert_type(w & jnp.uint32(0xFFFF0000), f32)


def _bfly_fwd(a):
    (a0r, a0i), (a1r, a1i), (a2r, a2i), (a3r, a3i) = a
    t0r, t0i, t1r, t1i = a0r + a2r, a0i + a2i, a0r - a2r, a0i - a2i
    t2r, t2i, t3r, t3i = a1r + a3r, a1i + a3i, a1r - a3r, a1i - a3i
    return [(t0r + t2r, t0i + t2i), (t1r - t3i, t1i + t3r), (t0r - t2r, t0i - t2i), (t1r + t3i, t1i - t3r)]


def _bfly_inv(q):
    (q0r, q0i), (q1r, q1i), (q2r, q2i), (q3r, q3i) = q
    u0r, u0i, u1r, u1i = q0r + q2r, q0i + q2i, q0r - q2r, q0i - q2i
    u2r, u2i, u3r, u3i = q1r + q3r, q1i + q3i, q1r - q3r, q1i - q3i
    return [(u0r + u2r, u0i + u2i), (u1r + u3i, u1i - u3r), (u0r - u2r, u0i - u2i), (u1r - u3i, u1i + u3r)]


def interleave(main, nmain, sides):
    done = [0] * len(sides)
    i = 0
    for _ in main:
        i += 1
        f = i / nmain
        for s, (g, n, a, b) in enumerate(sides):
            want = min(n, max(0, int(np.ceil((f - a) / (b - a) * n - 1e-9))))
            while done[s] < want:
                next(g)
                done[s] += 1
    for s, (g, n, a, b) in enumerate(sides):
        while done[s] < n:
            next(g)
            done[s] += 1
        for _ in g:
            pass


class _NoScope:
    def __init__(self, name):
        pass

    def __enter__(self):
        return self

    def __exit__(self, *a):
        return False


def kernel(q_hbm, k_hbm, v_hbm, skt_ref, ssmk_hbm, ssmd_ref, wg_hbm, wu_hbm, wd_hbm, c_ref, wmod_hbm,
           F_hbm, Fi_hbm, o_hbm, F_ref, Fi_ref, sd_s,
           k_s, v_s, ssmk_s, kt_s, xs, gs, qs, y_s, q_s, wg_s, wu_s, wd_s, wmod_s, mod_s,
           x1_s, h2_s, hh_s, o_s, sems, osems):
    scope = jax.named_scope if SCOPES else _NoScope

    def conv_copy(c, i):
        c0 = c * 128 if isinstance(c, int) else pl.multiple_of(c * 128, 128)
        if i == 0:
            return pltpu.make_async_copy(ssmk_hbm.at[pl.ds(c0, 128), :], ssmk_s.at[c], sems.at[c])
        if i == 1:
            return pltpu.make_async_copy(k_hbm.at[:, pl.ds(c0, 128)], k_s.at[c, pl.ds(16, S), :], sems.at[NT + c])
        return pltpu.make_async_copy(v_hbm.at[:, pl.ds(c0, 128)], v_s.at[c], sems.at[2 * NT + c])

    nsem = [3 * NT + NB]

    def cp(src, dst):
        nsem[0] += 1
        return pltpu.make_async_copy(src, dst, sems.at[nsem[0] - 1])
    F_cp = cp(F_hbm, F_ref)
    Fi_cp = cp(Fi_hbm, Fi_ref)
    wmod_cps = [cp(wmod_hbm.at[i * 128:(i + 1) * 128, 0:5 * D], wmod_s.at[i * 128:(i + 1) * 128, 0:5 * D]) for i in range(NT)]
    gb_cp = cp(wmod_hbm.at[:, 5 * D:6 * D], wmod_s.at[:, 5 * D:6 * D])
    WP = 256
    wg_cps = [cp(wg_hbm.at[:, n * WP:(n + 1) * WP], wg_s.at[:, n * WP:(n + 1) * WP]) for n in range(F // WP)]
    wu_cps = [cp(wu_hbm.at[:, n * WP:(n + 1) * WP], wu_s.at[:, n * WP:(n + 1) * WP]) for n in range(F // WP)]
    wd_cps = [cp(wd_hbm.at[:, n * 128:(n + 1) * 128], wd_s.at[:, n * 128:(n + 1) * 128]) for n in range(NT)]

    def q_copy(b):
        r0 = b * MB if isinstance(b, int) else pl.multiple_of(b * MB, MB)
        return pltpu.make_async_copy(q_hbm.at[pl.ds(r0, MB), :], q_s.at[pl.ds(r0, MB), :], sems.at[3 * NT + b])

    base0 = nsem[0]
    nsem[0] += 3 * NC

    def chunk_copy(j, i):
        r0 = j * L if isinstance(j, int) else pl.multiple_of(j * L, L)
        r16 = 16 + r0 if isinstance(j, int) else pl.multiple_of(16 + r0, 16)
        sem = sems.at[base0 + i * NC + j]
        if i == 0:
            return pltpu.make_async_copy(ssmk_hbm.at[0:128, pl.ds(r0, L)], ssmk_s.at[0, :, pl.ds(r0, L)], sem)
        if i == 1:
            return pltpu.make_async_copy(k_hbm.at[pl.ds(r0, L), 0:128], k_s.at[0, pl.ds(r16, L), :], sem)
        return pltpu.make_async_copy(v_hbm.at[pl.ds(r0, L), 0:128], v_s.at[0, pl.ds(r0, L), :], sem)
    for j in range(NC):
        chunk_copy(j, 0).start()
        if j == 0:
            F_cp.start()
        chunk_copy(j, 1).start()
        chunk_copy(j, 2).start()
    Fi_cp.start()
    for c in range(1, NT):
        for i in range(3):
            conv_copy(c, i).start()

    def start_late():
        for d in wmod_cps:
            d.start()
        q_copy(0).start()
        for n in range(F // WP):
            wg_cps[n].start()
            wu_cps[n].start()
            if n == 2:
                q_copy(1).start()
        gb_cp.start()
        for d in wd_cps:
            d.start()
        for b in range(2, NB):
            q_copy(b).start()

    sd_s[...] = ssmd_ref[...].astype(f32).reshape(1, D)
    for c in range(NT):
        k_s[c, 0:16, :] = jnp.zeros((16, 128), bf16)

    def T_tile(c, t):
        t0 = t * 128 if isinstance(t, int) else pl.multiple_of(t * 128, 128)
        kt_s[pl.ds(t0, 128), :] = ssmk_s[c, :, pl.ds(t0, 128)].T

    def phases(wref, off):
        a = wref[pl.ds(off, 128, stride=2), :]
        b = wref[pl.ds(off + 1, 128, stride=2), :]
        return [_lo(a), _hi(a), _lo(b), _hi(b)]

    def spectrum(parts, dst, j, first, extra=None):
        for g in range(16):
            a = [(parts[r][16 * g:16 * g + 8], parts[r][16 * g + 8:16 * g + 16]) for r in range(4)]
            if extra is not None:
                a[0] = (a[0][0] + extra, a[0][1])
            for q, (re, im) in enumerate(_bfly_fwd(a)):
                if first:
                    trip = (re + im, re, im)
                else:
                    trip = (re, im - re, re + im)
                for u in range(3):
                    dst[j, q, u, 8 * g:8 * g + 8, :] = trip[u]

    def F_chunk(c, j):
        c0 = pl.multiple_of(c * 128, 128) if not isinstance(c, int) else c * 128
        w0 = j * (L // 2) if isinstance(j, int) else pl.multiple_of(j * (L // 2), L // 2)
        kk = phases(kt_s.bitcast(u32).at[pl.ds(w0, L // 2), :], 0)
        kparts = [jnp.dot(F_ref[r], kk[r].astype(bf16), preferred_element_type=f32) for r in range(4)]
        w = skt_ref[:, pl.ds(c0, 128)].astype(f32)
        kw = k_s.bitcast(u32).at[c, pl.ds(w0, L // 2 + 8), :]
        vw = v_s.bitcast(u32).at[c, pl.ds(w0, L // 2), :]
        kc = phases(kw, 8)
        kp = phases(kw, 6)
        vv = phases(vw, 0)
        taps = [[kc[0], kp[3], kp[2], kp[1]], [kc[1], kc[0], kp[3], kp[2]],
                [kc[2], kc[1], kc[0], kp[3]], [kc[3], kc[2], kc[1], kc[0]]]
        parts = []
        for r in range(4):
            ks = taps[r][0] * w[0:1] + taps[r][1] * w[1:2] + taps[r][2] * w[2:3] + taps[r][3] * w[3:4]
            kv = (ks * vv[r]).astype(bf16)
            parts.append(jnp.dot(F_ref[r], kv, preferred_element_type=f32))
        sd = jnp.where(j == 0, sd_s[:, pl.ds(c0, 128)], 0.0)
        spectrum(kparts, gs, j, False, extra=sd)
        spectrum(parts, xs, j, True)

    def C_pos(p):
        r0 = pl.multiple_of(p * 8, 8)
        for q in range(4):
            X = [tuple(xs[j, q, u, pl.ds(r0, 8), :] for u in range(3)) for j in range(NC)]
            G = [tuple(gs[m, q, u, pl.ds(r0, 8), :] for u in range(3)) for m in range(NC)]
            prev = None
            for i in range(NC):
                acc = None
                for j in range(i + 1):
                    s, xr, xi = X[j]
                    gr, d, t = G[i - j]
                    q3 = (gr * s, xr * d, xi * t)
                    acc = q3 if acc is None else (acc[0] + q3[0], acc[1] + q3[1], acc[2] + q3[2])
                pr, pi = acc[0] - acc[2], acc[0] + acc[1]
                qr, qi = (pr, pi) if prev is None else (pr + prev[1], pi - prev[0])
                prev = (pr, pi)
                qs[i, q, 0, pl.ds(r0, 8), :] = qr
                qs[i, q, 1, pl.ds(r0, 8), :] = qi

    def I_chunk(c, j):
        r0 = j * L if isinstance(j, int) else pl.multiple_of(j * L, L)
        yv = y_s.at[c, pl.ds(r0, L), :]
        rows = [[] for _ in range(4)]
        for g in range(16):
            Q = [(qs[j, q, 0, 8 * g:8 * g + 8, :], qs[j, q, 1, 8 * g:8 * g + 8, :]) for q in range(4)]
            for r, (br, bi) in enumerate(_bfly_inv(Q)):
                rows[r].append(jnp.concatenate([br, bi], axis=0).astype(bf16))
        for r in range(4):
            yv[pl.ds(r, 128, stride=4), :] = jnp.dot(Fi_ref[r], jnp.concatenate(rows[r], axis=0),
                                                     preferred_element_type=f32)

    def loop(n, fn):
        def body(i, carry):
            fn(i)
            return carry
        lax.fori_loop(0, n, body, 0)

    def C_iter(po):
        for u in range(CU):
            C_pos(po * CU + u)

    def mod_part(i):
        wmod_cps[i].wait()
        cf = c_ref[:, i * 128:(i + 1) * 128].astype(f32)
        sc = (cf * jax.nn.sigmoid(cf)).astype(bf16)
        acc = jnp.dot(sc, wmod_s[i * 128:(i + 1) * 128, 0:5 * D], preferred_element_type=f32)
        if i > 0:
            acc = acc + mod_s[:, 0:5 * D]
        if i == NT - 1:
            acc = acc.astype(bf16).astype(f32)
        mod_s[:, 0:5 * D] = acc

    def mod_gb():
        cf = c_ref[...].astype(f32)
        sc = (cf * jax.nn.sigmoid(cf)).astype(bf16)
        mod_s[:, 5 * D:6 * D] = jnp.dot(sc, wmod_s[:, 5 * D:6 * D], preferred_element_type=f32).astype(bf16).astype(f32)

    def wait_T(j):
        chunk_copy(j, 0).wait()
        for t in range(4):
            T_tile(0, 4 * j + t)

    def first_F():
        wait_T(0)
        F_cp.wait()
        def body(j):
            chunk_copy(j, 1).wait()
            chunk_copy(j, 2).wait()
            F_chunk(0, j)
            pl.when(j + 1 < NC)(lambda: wait_T(j + 1))
        loop(NC, body)

    def I_loop(c):
        conv_copy(c + 1, 0).wait()
        def i_body(jo):
            for u in range(IU):
                I_chunk(c, jo * IU + u)
                for t in range(4):
                    T_tile(c + 1, (jo * IU + u) * 4 + t)
        loop(NC // IU, i_body)

    def mod_parts(c, parts):
        @pl.when(c == NT - 1)
        def _():
            for i in parts:
                mod_part(i)

    with scope("F0"):
        first_F()
        start_late()
    with scope("conv"):
        def tile_body(c):
            with scope("I"):
                I_loop(c - 1)
            with scope("wkv"):
                conv_copy(c, 1).wait()
                conv_copy(c, 2).wait()
            mod_parts(c, MOD_A)
            with scope("F"):
                def f_body(jo):
                    for u in range(FU):
                        F_chunk(c, jo * FU + u)
                loop(NC // FU, f_body)
            mod_parts(c, MOD_B)
            with scope("C"):
                loop(16 // CU, C_iter)
        loop(16 // CU, C_iter)
        Fi_cp.wait()
        def tb(c, carry):
            tile_body(c)
            return carry
        lax.fori_loop(1, NT, tb, 0)
        with scope("mod"):
            for i in range(MOD_B[-1] + 1, NT):
                mod_part(i)

    def pre_gen(b, slot):
        for p in range(MB // PR):
            r0 = b * MB + p * PR
            if not isinstance(r0, int):
                r0 = pl.multiple_of(r0, PR)
            sa = mod_s[:, 0 * D:1 * D]
            ca = mod_s[:, 1 * D:2 * D]
            ga = mod_s[:, 2 * D:3 * D]
            sb = mod_s[:, 3 * D:4 * D]
            cb = mod_s[:, 4 * D:5 * D]
            x = q_s[pl.ds(r0, PR), :].astype(f32)
            y = jnp.concatenate([y_s[c, pl.ds(r0, PR), :] for c in range(NT)], axis=1)
            h = _ln(x) * (1.0 + ca) + sa
            x1 = (x + ga * (h * y)).astype(bf16)
            x1_s[slot, p * PR:(p + 1) * PR, :] = x1
            x1 = x1.astype(f32)
            h2_s[slot, p * PR:(p + 1) * PR, :] = (_ln(x1) * (1.0 + cb) + sb).astype(bf16)
            yield

    def mlp_gen(slot, first=False, tails=None):
        for n in range(F // 128):
            cs = slice(n * 128, (n + 1) * 128)
            a = h2_s[slot]
            if first and n in GW:
                with scope("wgw"):
                    for i in range(n * 128 // WP, GW[n]):
                        wg_cps[i].wait()
                        wu_cps[i].wait()
                    if n == Q1W:
                        q_copy(1).wait()
            g = jnp.dot(a, wg_s[:, cs], preferred_element_type=f32)
            yield
            u = jnp.dot(a, wu_s[:, cs], preferred_element_type=f32)
            hh_s[:, cs] = (jnp.maximum(g, 0.0) * u).astype(bf16)
            yield
        for n in range(NT):
            cs = slice(n * 128, (n + 1) * 128)
            acc = None
            if first and n in DW:
                with scope("wdw"):
                    for i in range(n, DW[n]):
                        wd_cps[i].wait()
                    if n == 0:
                        gb_cp.wait()
            for kk in range(0, F // 128, KD):
                ks = slice(kk * 128, (kk + KD) * 128)
                d1 = jnp.dot(hh_s[:, ks], wd_s[ks, cs], preferred_element_type=f32)
                acc = d1 if acc is None else acc + d1
                if first and n == 0 and kk == 0:
                    mod_gb()
                if kk + KD >= F // 128:
                    gb = mod_s[:, 5 * D + n * 128:5 * D + (n + 1) * 128]
                    o_s[slot, :, cs] = (x1_s[slot, :, cs].astype(f32) + gb * acc).astype(bf16)
                    if tails is not None:
                        tails[n].start()
                yield
    NM = 2 * (F // 128) + NT * (F // 128 // KD)

    def out_copy(b, slot):
        return pltpu.make_async_copy(o_s.at[slot], o_hbm.at[pl.ds(pl.multiple_of(b * MB, MB), MB), :], osems.at[slot])

    def i_gen(c, chunks):
        for j in chunks:
            I_chunk(c, j)
            yield

    with scope("pre0"):
        I_chunk(NT - 1, 0)
        q_copy(0).wait()
        for _ in pre_gen(0, 0):
            pass
    with scope("blk0"):
        interleave(mlp_gen(0, first=True), NM, [(i_gen(NT - 1, range(1, NC)), NC - 1, IA, IB),
                                                (pre_gen(1, 1), MB // PR, PA, 0.95)])
        out_copy(0, 0).start()

    with scope("main"):
        def main_body(b, carry):
            slot = b % 2
            @pl.when(b >= 2)
            def _():
                out_copy(b - 2, slot).wait()
            q_copy(b + 1).wait()
            interleave(mlp_gen(slot), NM, [(pre_gen(b + 1, 1 - slot), MB // PR, 0.0, 0.95)])
            out_copy(b, slot).start()
            return carry
        lax.fori_loop(1, NB - 1, main_body, 0)
    with scope("last"):
        lb, lp = NB - 1, (NB - 1) % 2
        out_copy(NB - 3, (NB - 3) % 2).wait()
        tails = [pltpu.make_async_copy(o_s.at[lp, :, n * 128:(n + 1) * 128],
                                       o_hbm.at[lb * MB:(lb + 1) * MB, n * 128:(n + 1) * 128], osems.at[2 + n])
                 for n in range(NT)]
        for _ in mlp_gen(lp, tails=tails):
            pass
    with scope("tail"):
        out_copy(NB - 2, (NB - 2) % 2).wait()
        for d in tails:
            d.wait()


@jax.jit
def pallas_adaLN_cond__ssm_conv_h3__glu_gated_reglu__prompt_kernel(
        A_q, A_k, A_v, A_shift_k, A_ssm_k, A_ssm_D, B_x, B_W_gate, B_W_up, B_W_down, c, w_mod):
    Fm, Fi = _dft_consts()
    Fm = jnp.asarray(Fm.astype(np.float32)).astype(bf16)
    Fi = jnp.asarray(Fi.astype(np.float32)).astype(bf16)
    hbm = pl.BlockSpec(memory_space=pl.ANY)
    vm = pl.BlockSpec(memory_space=pltpu.VMEM)
    out = pl.pallas_call(
        kernel,
        out_shape=jax.ShapeDtypeStruct((S, D), A_q.dtype),
        in_specs=[hbm, hbm, hbm, vm, hbm, vm, hbm, hbm, hbm, vm, hbm, hbm, hbm],
        out_specs=hbm,
        scratch_shapes=[
            pltpu.VMEM((4, 256, 128), bf16),
            pltpu.VMEM((4, 128, 256), bf16),
            pltpu.VMEM((1, D), f32),
            pltpu.VMEM((NT, S + 16, 128), bf16),
            pltpu.VMEM((NT, S, 128), bf16),
            pltpu.VMEM((NT, 128, S), bf16),
            pltpu.VMEM((S, 128), bf16),
            pltpu.VMEM((NC, 4, 3, 128 + PAD, 128), f32),
            pltpu.VMEM((NC, 4, 3, 128 + PAD, 128), f32),
            pltpu.VMEM((NC, 4, 2, 128 + PAD, 128), f32),
            pltpu.VMEM((NT, S + PAD, 128), f32),
            pltpu.VMEM((S, D), bf16),
            pltpu.VMEM((D, F), bf16),
            pltpu.VMEM((D, F), bf16),
            pltpu.VMEM((F, D), bf16),
            pltpu.VMEM((D, 6 * D), bf16),
            pltpu.VMEM((1, 6 * D), f32),
            pltpu.VMEM((2, MB, D), bf16),
            pltpu.VMEM((2, MB, D), bf16),
            pltpu.VMEM((MB, F), bf16),
            pltpu.VMEM((2, MB, D), bf16),
            pltpu.SemaphoreType.DMA((3 * NT + NB + 3 + 2 * (F // 256) + 2 * NT + 3 * NC,)),
            pltpu.SemaphoreType.DMA((2 + NT,)),
        ],
        compiler_params=pltpu.CompilerParams(vmem_limit_bytes=120 * 1024 * 1024),
    )(A_q.reshape(S, D), A_k.reshape(S, D), A_v.reshape(S, D), A_shift_k.T, A_ssm_k, A_ssm_D,
      B_W_gate, B_W_up, B_W_down, c, w_mod, Fm, Fi)
    return out.reshape(A_q.shape)
```

```python
import numpy as np
import jax
import jax.numpy as jnp
from jax import lax
import jax.experimental.pallas as pl
import jax.experimental.pallas.tpu as pltpu

S, D, F = 2048, 640, 1536
L = 512
NC = S // L
NT = D // 128
MB = 256
NB = S // MB
PR = 16
KD = 4
FU = 4
IU = 4
CU = 4
GW = {0: 1, 4: 2, 8: 3}
DW = {0: 1, 2: 2}
WP = 512
DP = (0, 2, 5)
LATE_AT = 0
PAD = 8
MOD_A, MOD_B = (0, 0), (0, 0)
Q1W, Q1S = 4, 0
IA, IB, PA = 0.0, 0.18, 0.24
SCOPES = False
f32, bf16, u32 = jnp.float32, jnp.bfloat16, jnp.uint32


def _ln(x):
    m = jnp.sum(x, axis=-1, keepdims=True) * (1.0 / D)
    xc = x - m
    v = jnp.sum(xc * xc, axis=-1, keepdims=True) * (1.0 / D)
    return xc * lax.rsqrt(v + 1e-5)


def _lo(w):
    return lax.bitcast_convert_type(w << 16, f32)


def _hi(w):
    return lax.bitcast_convert_type(w & jnp.uint32(0xFFFF0000), f32)


def _bfly_fwd(a):
    (a0r, a0i), (a1r, a1i), (a2r, a2i), (a3r, a3i) = a
    t0r, t0i, t1r, t1i = a0r + a2r, a0i + a2i, a0r - a2r, a0i - a2i
    t2r, t2i, t3r, t3i = a1r + a3r, a1i + a3i, a1r - a3r, a1i - a3i
    return [(t0r + t2r, t0i + t2i), (t1r - t3i, t1i + t3r), (t0r - t2r, t0i - t2i), (t1r + t3i, t1i - t3r)]


def _bfly_inv(q):
    (q0r, q0i), (q1r, q1i), (q2r, q2i), (q3r, q3i) = q
    u0r, u0i, u1r, u1i = q0r + q2r, q0i + q2i, q0r - q2r, q0i - q2i
    u2r, u2i, u3r, u3i = q1r + q3r, q1i + q3i, q1r - q3r, q1i - q3i
    return [(u0r + u2r, u0i + u2i), (u1r + u3i, u1i - u3r), (u0r - u2r, u0i - u2i), (u1r - u3i, u1i + u3r)]


def interleave(main, nmain, sides):
    done = [0] * len(sides)
    i = 0
    for _ in main:
        i += 1
        f = i / nmain
        for s, (g, n, a, b) in enumerate(sides):
            want = min(n, max(0, int(np.ceil((f - a) / (b - a) * n - 1e-9))))
            while done[s] < want:
                next(g)
                done[s] += 1
    for s, (g, n, a, b) in enumerate(sides):
        while done[s] < n:
            next(g)
            done[s] += 1
        for _ in g:
            pass


class _NoScope:
    def __init__(self, name):
        pass

    def __enter__(self):
        return self

    def __exit__(self, *a):
        return False


def kernel(q_hbm, k_hbm, v_hbm, skt_ref, ssmk_hbm, ssmd_ref, wg_hbm, wu_hbm, wd_hbm, c_ref, wmod_hbm,
           F0_hbm, o_hbm, F0_ref, F_ref, Fi_ref, sd_s,
           k_s, v_s, ssmk_s, kt_s, xs, gs, qs, y_s, q_s, wg_s, wu_s, wd_s, wmod_s, mod_s,
           x1_s, h2_s, hh_s, o_s, sems, osems):
    scope = jax.named_scope if SCOPES else _NoScope

    def conv_copy(c, i):
        c0 = c * 128 if isinstance(c, int) else pl.multiple_of(c * 128, 128)
        if i == 0:
            return pltpu.make_async_copy(ssmk_hbm.at[pl.ds(c0, 128), :], ssmk_s.at[c], sems.at[c])
        if i == 1:
            return pltpu.make_async_copy(k_hbm.at[:, pl.ds(c0, 128)], k_s.at[c, pl.ds(16, S), :], sems.at[NT + c])
        return pltpu.make_async_copy(v_hbm.at[:, pl.ds(c0, 128)], v_s.at[c], sems.at[2 * NT + c])

    nsem = [3 * NT + NB]

    def cp(src, dst):
        nsem[0] += 1
        return pltpu.make_async_copy(src, dst, sems.at[nsem[0] - 1])
    wmod_cps = [cp(wmod_hbm.at[i * 128:(i + 1) * 128, 0:5 * D], wmod_s.at[i * 128:(i + 1) * 128, 0:5 * D]) for i in range(NT)]
    gb_cp = cp(wmod_hbm.at[:, 5 * D:6 * D], wmod_s.at[:, 5 * D:6 * D])
    wg_cps = [cp(wg_hbm.at[:, n * WP:(n + 1) * WP], wg_s.at[:, n * WP:(n + 1) * WP]) for n in range(F // WP)]
    wu_cps = [cp(wu_hbm.at[:, n * WP:(n + 1) * WP], wu_s.at[:, n * WP:(n + 1) * WP]) for n in range(F // WP)]
    wd_cps = [cp(wd_hbm.at[:, a * 128:b * 128], wd_s.at[:, a * 128:b * 128]) for a, b in zip(DP[:-1], DP[1:])]

    def q_copy(b):
        r0 = b * MB if isinstance(b, int) else pl.multiple_of(b * MB, MB)
        return pltpu.make_async_copy(q_hbm.at[pl.ds(r0, MB), :], q_s.at[pl.ds(r0, MB), :], sems.at[3 * NT + b])

    F0_cp = cp(F0_hbm, F0_ref)
    F0_cp.start()
    base0 = nsem[0]
    nsem[0] += 3 * NC

    def chunk_copy(j, i):
        r0 = j * L if isinstance(j, int) else pl.multiple_of(j * L, L)
        r16 = 16 + r0 if isinstance(j, int) else pl.multiple_of(16 + r0, 16)
        sem = sems.at[base0 + i * NC + j]
        if i == 0:
            return pltpu.make_async_copy(ssmk_hbm.at[0:128, pl.ds(r0, L)], ssmk_s.at[0, :, pl.ds(r0, L)], sem)
        if i == 1:
            return pltpu.make_async_copy(k_hbm.at[pl.ds(r0, L), 0:128], k_s.at[0, pl.ds(r16, L), :], sem)
        return pltpu.make_async_copy(v_hbm.at[pl.ds(r0, L), 0:128], v_s.at[0, pl.ds(r0, L), :], sem)
    for j in range(NC):
        chunk_copy(j, 0).start()
        chunk_copy(j, 1).start()
        chunk_copy(j, 2).start()
    for c in range(1, NT):
        for i in range(3):
            conv_copy(c, i).start()

    def start_late():
        for d in wmod_cps:
            d.start()
        q_copy(0).start()
        for n in range(F // WP):
            wg_cps[n].start()
            wu_cps[n].start()
            if n == Q1S:
                q_copy(1).start()
        gb_cp.start()
        for d in wd_cps:
            d.start()
        for b in range(2, NB):
            q_copy(b).start()

    ki = lax.broadcasted_iota(jnp.int32, (128, 128), 0)
    ang = (4 * ki + 1).astype(f32) * (2.0 * np.pi / (4 * L))
    twr, twi = jnp.cos(ang), jnp.sin(ang)
    F0_cp.wait()
    co, si = F0_ref[0:128], F0_ref[128:256]
    for r in range(4):
        if r > 0:
            co, si = co * twr - si * twi, co * twi + si * twr
        fr = jnp.concatenate([t[8 * g:8 * g + 8] for g in range(16) for t in (co, si)], axis=0)
        F_ref[r] = fr.astype(bf16)
        Fi_ref[r] = (fr * (1.0 / L)).astype(bf16).T

    sd_s[...] = ssmd_ref[...].astype(f32).reshape(1, D)
    for c in range(NT):
        k_s[c, 0:16, :] = jnp.zeros((16, 128), bf16)

    def T_tile(c, t):
        t0 = t * 128 if isinstance(t, int) else pl.multiple_of(t * 128, 128)
        kt_s[pl.ds(t0, 128), :] = ssmk_s[c, :, pl.ds(t0, 128)].T

    def phases(wref, off):
        a = wref[pl.ds(off, 128, stride=2), :]
        b = wref[pl.ds(off + 1, 128, stride=2), :]
        return [_lo(a), _hi(a), _lo(b), _hi(b)]

    def spectrum(parts, dst, j, first, extra=None):
        for g in range(16):
            a = [(parts[r][16 * g:16 * g + 8], parts[r][16 * g + 8:16 * g + 16]) for r in range(4)]
            if extra is not None:
                a[0] = (a[0][0] + extra, a[0][1])
            for q, (re, im) in enumerate(_bfly_fwd(a)):
                if first:
                    trip = (re + im, re, im)
                else:
                    trip = (re, im - re, re + im)
                for u in range(3):
                    dst[j, q, u, 8 * g:8 * g + 8, :] = trip[u]

    def F_chunk(c, j):
        c0 = pl.multiple_of(c * 128, 128) if not isinstance(c, int) else c * 128
        w0 = j * (L // 2) if isinstance(j, int) else pl.multiple_of(j * (L // 2), L // 2)
        kk = phases(kt_s.bitcast(u32).at[pl.ds(w0, L // 2), :], 0)
        kparts = [jnp.dot(F_ref[r], kk[r].astype(bf16), preferred_element_type=f32) for r in range(4)]
        w = skt_ref[:, pl.ds(c0, 128)].astype(f32)
        kw = k_s.bitcast(u32).at[c, pl.ds(w0, L // 2 + 8), :]
        vw = v_s.bitcast(u32).at[c, pl.ds(w0, L // 2), :]
        kc = phases(kw, 8)
        kp = phases(kw, 6)
        vv = phases(vw, 0)
        taps = [[kc[0], kp[3], kp[2], kp[1]], [kc[1], kc[0], kp[3], kp[2]],
                [kc[2], kc[1], kc[0], kp[3]], [kc[3], kc[2], kc[1], kc[0]]]
        parts = []
        for r in range(4):
            ks = taps[r][0] * w[0:1] + taps[r][1] * w[1:2] + taps[r][2] * w[2:3] + taps[r][3] * w[3:4]
            kv = (ks * vv[r]).astype(bf16)
            parts.append(jnp.dot(F_ref[r], kv, preferred_element_type=f32))
        sd = jnp.where(j == 0, sd_s[:, pl.ds(c0, 128)], 0.0)
        spectrum(kparts, gs, j, False, extra=sd)
        spectrum(parts, xs, j, True)

    def C_pos(p):
        r0 = pl.multiple_of(p * 8, 8)
        for q in range(4):
            X = [tuple(xs[j, q, u, pl.ds(r0, 8), :] for u in range(3)) for j in range(NC)]
            G = [tuple(gs[m, q, u, pl.ds(r0, 8), :] for u in range(3)) for m in range(NC)]
            prev = None
            for i in range(NC):
                acc = None
                for j in range(i + 1):
                    s, xr, xi = X[j]
                    gr, d, t = G[i - j]
                    q3 = (gr * s, xr * d, xi * t)
                    acc = q3 if acc is None else (acc[0] + q3[0], acc[1] + q3[1], acc[2] + q3[2])
                pr, pi = acc[0] - acc[2], acc[0] + acc[1]
                qr, qi = (pr, pi) if prev is None else (pr + prev[1], pi - prev[0])
                prev = (pr, pi)
                qs[i, q, 0, pl.ds(r0, 8), :] = qr
                qs[i, q, 1, pl.ds(r0, 8), :] = qi

    def I_chunk(c, j):
        r0 = j * L if isinstance(j, int) else pl.multiple_of(j * L, L)
        yv = y_s.at[c, pl.ds(r0, L), :]
        rows = [[] for _ in range(4)]
        for g in range(16):
            Q = [(qs[j, q, 0, 8 * g:8 * g + 8, :], qs[j, q, 1, 8 * g:8 * g + 8, :]) for q in range(4)]
            for r, (br, bi) in enumerate(_bfly_inv(Q)):
                rows[r].append(jnp.concatenate([br, bi], axis=0).astype(bf16))
        for r in range(4):
            yv[pl.ds(r, 128, stride=4), :] = jnp.dot(Fi_ref[r], jnp.concatenate(rows[r], axis=0),
                                                     preferred_element_type=f32)

    def loop(n, fn):
        def body(i, carry):
            fn(i)
            return carry
        lax.fori_loop(0, n, body, 0)

    def C_iter(po):
        for u in range(CU):
            C_pos(po * CU + u)

    def mod_part(i0, i1):
        for i in range(i0, i1):
            wmod_cps[i].wait()
        cf = c_ref[:, i0 * 128:i1 * 128].astype(f32)
        sc = (cf * jax.nn.sigmoid(cf)).astype(bf16)
        acc = jnp.dot(sc, wmod_s[i0 * 128:i1 * 128, 0:5 * D], preferred_element_type=f32)
        if i0 > 0:
            acc = acc + mod_s[:, 0:5 * D]
        if i1 == NT:
            acc = acc.astype(bf16).astype(f32)
        mod_s[:, 0:5 * D] = acc

    def mod_gb():
        cf = c_ref[...].astype(f32)
        sc = (cf * jax.nn.sigmoid(cf)).astype(bf16)
        mod_s[:, 5 * D:6 * D] = jnp.dot(sc, wmod_s[:, 5 * D:6 * D], preferred_element_type=f32).astype(bf16).astype(f32)

    def wait_T(j):
        chunk_copy(j, 0).wait()
        for t in range(4):
            T_tile(0, 4 * j + t)

    def first_F():
        wait_T(0)
        def body(j):
            chunk_copy(j, 1).wait()
            chunk_copy(j, 2).wait()
            F_chunk(0, j)
            pl.when(j + 1 < NC)(lambda: wait_T(j + 1))
        loop(NC, body)

    def I_loop(c):
        conv_copy(c + 1, 0).wait()
        def i_body(jo):
            for u in range(IU):
                I_chunk(c, jo * IU + u)
                for t in range(4):
                    T_tile(c + 1, (jo * IU + u) * 4 + t)
        loop(NC // IU, i_body)

    def mod_parts(c, parts):
        if parts[1] > parts[0]:
            pl.when(c == NT - 1)(lambda: mod_part(*parts))

    with scope("F0"):
        first_F()
        start_late()
    with scope("conv"):
        def tile_body(c):
            with scope("I"):
                I_loop(c - 1)
            with scope("wkv"):
                conv_copy(c, 1).wait()
                conv_copy(c, 2).wait()
            mod_parts(c, MOD_A)
            with scope("F"):
                def f_body(jo):
                    for u in range(FU):
                        F_chunk(c, jo * FU + u)
                loop(NC // FU, f_body)
            mod_parts(c, MOD_B)
            with scope("C"):
                loop(16 // CU, C_iter)
        loop(16 // CU, C_iter)
        def tb(c, carry):
            tile_body(c)
            return carry
        lax.fori_loop(1, NT, tb, 0)
        with scope("mod"):
            if MOD_B[1] < NT:
                mod_part(MOD_B[1], NT)

    def pre_gen(b, slot):
        for p in range(MB // PR):
            r0 = b * MB + p * PR
            if not isinstance(r0, int):
                r0 = pl.multiple_of(r0, PR)
            sa = mod_s[:, 0 * D:1 * D]
            ca = mod_s[:, 1 * D:2 * D]
            ga = mod_s[:, 2 * D:3 * D]
            sb = mod_s[:, 3 * D:4 * D]
            cb = mod_s[:, 4 * D:5 * D]
            x = q_s[pl.ds(r0, PR), :].astype(f32)
            y = jnp.concatenate([y_s[c, pl.ds(r0, PR), :] for c in range(NT)], axis=1)
            h = _ln(x) * (1.0 + ca) + sa
            x1 = (x + ga * (h * y)).astype(bf16)
            x1_s[slot, p * PR:(p + 1) * PR, :] = x1
            x1 = x1.astype(f32)
            h2_s[slot, p * PR:(p + 1) * PR, :] = (_ln(x1) * (1.0 + cb) + sb).astype(bf16)
            yield

    def mlp_gen(slot, first=False, tails=None):
        for n in range(F // 128):
            cs = slice(n * 128, (n + 1) * 128)
            a = h2_s[slot]
            if first and n in GW:
                with scope("wgw"):
                    for i in range(n * 128 // WP, GW[n]):
                        wg_cps[i].wait()
                        wu_cps[i].wait()
                    if n == Q1W:
                        q_copy(1).wait()
            g = jnp.dot(a, wg_s[:, cs], preferred_element_type=f32)
            yield
            u = jnp.dot(a, wu_s[:, cs], preferred_element_type=f32)
            hh_s[:, cs] = (jnp.maximum(g, 0.0) * u).astype(bf16)
            yield
        for n in range(NT):
            cs = slice(n * 128, (n + 1) * 128)
            acc = None
            if first and n in DW:
                with scope("wdw"):
                    wd_cps[DW[n] - 1].wait()
                    if n == 0:
                        gb_cp.wait()
            for kk in range(0, F // 128, KD):
                ks = slice(kk * 128, (kk + KD) * 128)
                d1 = jnp.dot(hh_s[:, ks], wd_s[ks, cs], preferred_element_type=f32)
                acc = d1 if acc is None else acc + d1
                if first and n == 0 and kk == 0:
                    mod_gb()
                if kk + KD >= F // 128:
                    gb = mod_s[:, 5 * D + n * 128:5 * D + (n + 1) * 128]
                    o_s[slot, :, cs] = (x1_s[slot, :, cs].astype(f32) + gb * acc).astype(bf16)
                    if tails is not None:
                        tails[n].start()
                yield
    NM = 2 * (F // 128) + NT * (F // 128 // KD)

    def out_copy(b, slot):
        return pltpu.make_async_copy(o_s.at[slot], o_hbm.at[pl.ds(pl.multiple_of(b * MB, MB), MB), :], osems.at[slot])

    def i_gen(c, chunks):
        for j in chunks:
            I_chunk(c, j)
            yield

    with scope("pre0"):
        I_chunk(NT - 1, 0)
        q_copy(0).wait()
        for _ in pre_gen(0, 0):
            pass
    with scope("blk0"):
        interleave(mlp_gen(0, first=True), NM, [(i_gen(NT - 1, range(1, NC)), NC - 1, IA, IB),
                                                (pre_gen(1, 1), MB // PR, PA, 0.95)])
        out_copy(0, 0).start()

    with scope("main"):
        def main_body(b, carry):
            slot = b % 2
            @pl.when(b >= 2)
            def _():
                out_copy(b - 2, slot).wait()
            q_copy(b + 1).wait()
            interleave(mlp_gen(slot), NM, [(pre_gen(b + 1, 1 - slot), MB // PR, 0.0, 0.95)])
            out_copy(b, slot).start()
            return carry
        lax.fori_loop(1, NB - 1, main_body, 0)
    with scope("last"):
        lb, lp = NB - 1, (NB - 1) % 2
        out_copy(NB - 3, (NB - 3) % 2).wait()
        tails = [pltpu.make_async_copy(o_s.at[lp, :, n * 128:(n + 1) * 128],
                                       o_hbm.at[lb * MB:(lb + 1) * MB, n * 128:(n + 1) * 128], osems.at[2 + n])
                 for n in range(NT)]
        for _ in mlp_gen(lp, tails=tails):
            pass
    with scope("tail"):
        out_copy(NB - 2, (NB - 2) % 2).wait()
        for d in tails:
            d.wait()


@jax.jit
def pallas_adaLN_cond__ssm_conv_h3__glu_gated_reglu__prompt_kernel(
        A_q, A_k, A_v, A_shift_k, A_ssm_k, A_ssm_D, B_x, B_W_gate, B_W_up, B_W_down, c, w_mod):
    ph = 2.0 * np.pi * (np.arange(128)[:, None] + 0.25) / 128 * np.arange(128)[None, :]
    F0 = jnp.asarray(np.concatenate([np.cos(ph), np.sin(ph)], axis=0).astype(np.float32))
    hbm = pl.BlockSpec(memory_space=pl.ANY)
    vm = pl.BlockSpec(memory_space=pltpu.VMEM)
    out = pl.pallas_call(
        kernel,
        out_shape=jax.ShapeDtypeStruct((S, D), A_q.dtype),
        in_specs=[hbm, hbm, hbm, vm, hbm, vm, hbm, hbm, hbm, vm, hbm, hbm],
        out_specs=hbm,
        scratch_shapes=[
            pltpu.VMEM((256, 128), f32),
            pltpu.VMEM((4, 256, 128), bf16),
            pltpu.VMEM((4, 128, 256), bf16),
            pltpu.VMEM((1, D), f32),
            pltpu.VMEM((NT, S + 16, 128), bf16),
            pltpu.VMEM((NT, S, 128), bf16),
            pltpu.VMEM((NT, 128, S), bf16),
            pltpu.VMEM((S, 128), bf16),
            pltpu.VMEM((NC, 4, 3, 128 + PAD, 128), f32),
            pltpu.VMEM((NC, 4, 3, 128 + PAD, 128), f32),
            pltpu.VMEM((NC, 4, 2, 128 + PAD, 128), f32),
            pltpu.VMEM((NT, S + PAD, 128), f32),
            pltpu.VMEM((S, D), bf16),
            pltpu.VMEM((D, F), bf16),
            pltpu.VMEM((D, F), bf16),
            pltpu.VMEM((F, D), bf16),
            pltpu.VMEM((D, 6 * D), bf16),
            pltpu.VMEM((1, 6 * D), f32),
            pltpu.VMEM((2, MB, D), bf16),
            pltpu.VMEM((2, MB, D), bf16),
            pltpu.VMEM((MB, F), bf16),
            pltpu.VMEM((2, MB, D), bf16),
            pltpu.SemaphoreType.DMA((3 * NT + NB + 2 + 2 * (F // WP) + NT + len(DP) - 1 + 3 * NC,)),
            pltpu.SemaphoreType.DMA((2 + NT,)),
        ],
        compiler_params=pltpu.CompilerParams(vmem_limit_bytes=120 * 1024 * 1024),
    )(A_q.reshape(S, D), A_k.reshape(S, D), A_v.reshape(S, D), A_shift_k.T, A_ssm_k, A_ssm_D,
      B_W_gate, B_W_up, B_W_down, c, w_mod, F0)
    return out.reshape(A_q.shape)
```

```python
import numpy as np
import jax
import jax.numpy as jnp
from jax import lax
import jax.experimental.pallas as pl
import jax.experimental.pallas.tpu as pltpu

S, D, F = 2048, 640, 1536
L = 512
NC = S // L
NT = D // 128
MB = 256
NB = S // MB
PR = 16
KD = 4
FU = 4
IU = 4
CU = 4
GW = {0: 1, 4: 2, 8: 3}
DW = {0: 1, 2: 2}
WP = 512
DP = (0, 2, 5)
PAD = 8
Q1W, Q1S = 4, 0
IA, IB, PA = 0.0, 0.18, 0.24
SCOPES = False
f32, bf16, u32 = jnp.float32, jnp.bfloat16, jnp.uint32


def _ln(x):
    m = jnp.sum(x, axis=-1, keepdims=True) * (1.0 / D)
    xc = x - m
    v = jnp.sum(xc * xc, axis=-1, keepdims=True) * (1.0 / D)
    return xc * lax.rsqrt(v + 1e-5)


def _lo(w):
    return lax.bitcast_convert_type(w << 16, f32)


def _hi(w):
    return lax.bitcast_convert_type(w & jnp.uint32(0xFFFF0000), f32)


def _bfly_fwd(a):
    (a0r, a0i), (a1r, a1i), (a2r, a2i), (a3r, a3i) = a
    t0r, t0i, t1r, t1i = a0r + a2r, a0i + a2i, a0r - a2r, a0i - a2i
    t2r, t2i, t3r, t3i = a1r + a3r, a1i + a3i, a1r - a3r, a1i - a3i
    return [(t0r + t2r, t0i + t2i), (t1r - t3i, t1i + t3r), (t0r - t2r, t0i - t2i), (t1r + t3i, t1i - t3r)]


def _bfly_inv(q):
    (q0r, q0i), (q1r, q1i), (q2r, q2i), (q3r, q3i) = q
    u0r, u0i, u1r, u1i = q0r + q2r, q0i + q2i, q0r - q2r, q0i - q2i
    u2r, u2i, u3r, u3i = q1r + q3r, q1i + q3i, q1r - q3r, q1i - q3i
    return [(u0r + u2r, u0i + u2i), (u1r + u3i, u1i - u3r), (u0r - u2r, u0i - u2i), (u1r - u3i, u1i + u3r)]


def interleave(main, nmain, sides):
    done = [0] * len(sides)
    i = 0
    for _ in main:
        i += 1
        f = i / nmain
        for s, (g, n, a, b) in enumerate(sides):
            want = min(n, max(0, int(np.ceil((f - a) / (b - a) * n - 1e-9))))
            while done[s] < want:
                next(g)
                done[s] += 1
    for s, (g, n, a, b) in enumerate(sides):
        while done[s] < n:
            next(g)
            done[s] += 1
        for _ in g:
            pass


class _NoScope:
    def __init__(self, name):
        pass

    def __enter__(self):
        return self

    def __exit__(self, *a):
        return False


def kernel(q_hbm, k_hbm, v_hbm, skt_hbm, ssmk_hbm, ssmd_hbm, wg_hbm, wu_hbm, wd_hbm, c_hbm, wmod_hbm,
           F0_hbm, o_hbm, skt_ref, ssmd_ref, c_ref, F0_ref, F_ref, Fi_ref, sd_s,
           k_s, v_s, ssmk_s, kt_s, xs, gs, qs, y_s, q_s, wg_s, wu_s, wd_s, wmod_s, mod_s,
           x1_s, h2_s, hh_s, o_s, sems, osems):
    scope = jax.named_scope if SCOPES else _NoScope

    def conv_copy(c, i):
        c0 = c * 128 if isinstance(c, int) else pl.multiple_of(c * 128, 128)
        if i == 0:
            return pltpu.make_async_copy(ssmk_hbm.at[pl.ds(c0, 128), :], ssmk_s.at[c], sems.at[c])
        if i == 1:
            return pltpu.make_async_copy(k_hbm.at[:, pl.ds(c0, 128)], k_s.at[c, pl.ds(16, S), :], sems.at[NT + c])
        return pltpu.make_async_copy(v_hbm.at[:, pl.ds(c0, 128)], v_s.at[c], sems.at[2 * NT + c])

    nsem = [3 * NT + NB]

    def cp(src, dst):
        nsem[0] += 1
        return pltpu.make_async_copy(src, dst, sems.at[nsem[0] - 1])
    wmod_cps = [cp(wmod_hbm.at[i * 128:(i + 1) * 128, 0:5 * D], wmod_s.at[i * 128:(i + 1) * 128, 0:5 * D]) for i in range(NT)]
    gb_cp = cp(wmod_hbm.at[:, 5 * D:6 * D], wmod_s.at[:, 5 * D:6 * D])
    wg_cps = [cp(wg_hbm.at[:, n * WP:(n + 1) * WP], wg_s.at[:, n * WP:(n + 1) * WP]) for n in range(F // WP)]
    wu_cps = [cp(wu_hbm.at[:, n * WP:(n + 1) * WP], wu_s.at[:, n * WP:(n + 1) * WP]) for n in range(F // WP)]
    wd_cps = [cp(wd_hbm.at[:, a * 128:b * 128], wd_s.at[:, a * 128:b * 128]) for a, b in zip(DP[:-1], DP[1:])]

    def q_copy(b):
        r0 = b * MB if isinstance(b, int) else pl.multiple_of(b * MB, MB)
        return pltpu.make_async_copy(q_hbm.at[pl.ds(r0, MB), :], q_s.at[pl.ds(r0, MB), :], sems.at[3 * NT + b])

    F0_cp = cp(F0_hbm, F0_ref)
    F0_cp.start()
    small_cps = [cp(skt_hbm, skt_ref), cp(ssmd_hbm, ssmd_ref), cp(c_hbm, c_ref)]
    for d in small_cps:
        d.start()
    base0 = nsem[0]
    nsem[0] += 3 * NC

    def chunk_copy(j, i):
        r0 = j * L if isinstance(j, int) else pl.multiple_of(j * L, L)
        r16 = 16 + r0 if isinstance(j, int) else pl.multiple_of(16 + r0, 16)
        sem = sems.at[base0 + i * NC + j]
        if i == 0:
            return pltpu.make_async_copy(ssmk_hbm.at[0:128, pl.ds(r0, L)], ssmk_s.at[0, :, pl.ds(r0, L)], sem)
        if i == 1:
            return pltpu.make_async_copy(k_hbm.at[pl.ds(r0, L), 0:128], k_s.at[0, pl.ds(r16, L), :], sem)
        return pltpu.make_async_copy(v_hbm.at[pl.ds(r0, L), 0:128], v_s.at[0, pl.ds(r0, L), :], sem)
    for j in range(NC):
        chunk_copy(j, 0).start()
        chunk_copy(j, 1).start()
        chunk_copy(j, 2).start()
    for c in range(1, NT):
        for i in range(3):
            conv_copy(c, i).start()

    def start_late():
        for d in wmod_cps:
            d.start()
        q_copy(0).start()
        for n in range(F // WP):
            wg_cps[n].start()
            wu_cps[n].start()
            if n == Q1S:
                q_copy(1).start()
        gb_cp.start()
        for d in wd_cps:
            d.start()
        for b in range(2, NB):
            q_copy(b).start()

    ki = lax.broadcasted_iota(jnp.int32, (128, 128), 0)
    ang = (4 * ki + 1).astype(f32) * (2.0 * np.pi / (4 * L))
    twr, twi = jnp.cos(ang), jnp.sin(ang)
    F0_cp.wait()
    co, si = F0_ref[0:128], F0_ref[128:256]
    for r in range(4):
        if r > 0:
            co, si = co * twr - si * twi, co * twi + si * twr
        fr = jnp.concatenate([t[8 * g:8 * g + 8] for g in range(16) for t in (co, si)], axis=0)
        F_ref[r] = fr.astype(bf16)
        Fi_ref[r] = (fr * (1.0 / L)).astype(bf16).T

    for d in small_cps:
        d.wait()
    sd_s[...] = ssmd_ref[...].astype(f32).reshape(1, D)
    for c in range(NT):
        k_s[c, 0:16, :] = jnp.zeros((16, 128), bf16)

    def T_tile(c, t):
        t0 = t * 128 if isinstance(t, int) else pl.multiple_of(t * 128, 128)
        kt_s[pl.ds(t0, 128), :] = ssmk_s[c, :, pl.ds(t0, 128)].T

    def phases(wref, off):
        a = wref[pl.ds(off, 128, stride=2), :]
        b = wref[pl.ds(off + 1, 128, stride=2), :]
        return [_lo(a), _hi(a), _lo(b), _hi(b)]

    def spectrum(parts, dst, j, first, extra=None):
        for g in range(16):
            a = [(parts[r][16 * g:16 * g + 8], parts[r][16 * g + 8:16 * g + 16]) for r in range(4)]
            if extra is not None:
                a[0] = (a[0][0] + extra, a[0][1])
            for q, (re, im) in enumerate(_bfly_fwd(a)):
                if first:
                    trip = (re + im, re, im)
                else:
                    trip = (re, im - re, re + im)
                for u in range(3):
                    dst[j, q, u, 8 * g:8 * g + 8, :] = trip[u]

    def F_chunk(c, j):
        c0 = pl.multiple_of(c * 128, 128) if not isinstance(c, int) else c * 128
        w0 = j * (L // 2) if isinstance(j, int) else pl.multiple_of(j * (L // 2), L // 2)
        kk = phases(kt_s.bitcast(u32).at[pl.ds(w0, L // 2), :], 0)
        kparts = [jnp.dot(F_ref[r], kk[r].astype(bf16), preferred_element_type=f32) for r in range(4)]
        w = skt_ref[:, pl.ds(c0, 128)].astype(f32)
        kw = k_s.bitcast(u32).at[c, pl.ds(w0, L // 2 + 8), :]
        vw = v_s.bitcast(u32).at[c, pl.ds(w0, L // 2), :]
        kc = phases(kw, 8)
        kp = phases(kw, 6)
        vv = phases(vw, 0)
        taps = [[kc[0], kp[3], kp[2], kp[1]], [kc[1], kc[0], kp[3], kp[2]],
                [kc[2], kc[1], kc[0], kp[3]], [kc[3], kc[2], kc[1], kc[0]]]
        parts = []
        for r in range(4):
            ks = taps[r][0] * w[0:1] + taps[r][1] * w[1:2] + taps[r][2] * w[2:3] + taps[r][3] * w[3:4]
            kv = (ks * vv[r]).astype(bf16)
            parts.append(jnp.dot(F_ref[r], kv, preferred_element_type=f32))
        sd = jnp.where(j == 0, sd_s[:, pl.ds(c0, 128)], 0.0)
        spectrum(kparts, gs, j, False, extra=sd)
        spectrum(parts, xs, j, True)

    def C_pos(p):
        r0 = pl.multiple_of(p * 8, 8)
        for q in range(4):
            X = [tuple(xs[j, q, u, pl.ds(r0, 8), :] for u in range(3)) for j in range(NC)]
            G = [tuple(gs[m, q, u, pl.ds(r0, 8), :] for u in range(3)) for m in range(NC)]
            prev = None
            for i in range(NC):
                acc = None
                for j in range(i + 1):
                    s, xr, xi = X[j]
                    gr, d, t = G[i - j]
                    q3 = (gr * s, xr * d, xi * t)
                    acc = q3 if acc is None else (acc[0] + q3[0], acc[1] + q3[1], acc[2] + q3[2])
                pr, pi = acc[0] - acc[2], acc[0] + acc[1]
                qr, qi = (pr, pi) if prev is None else (pr + prev[1], pi - prev[0])
                prev = (pr, pi)
                qs[i, q, 0, pl.ds(r0, 8), :] = qr
                qs[i, q, 1, pl.ds(r0, 8), :] = qi

    def I_chunk(c, j):
        r0 = j * L if isinstance(j, int) else pl.multiple_of(j * L, L)
        yv = y_s.at[c, pl.ds(r0, L), :]
        rows = [[] for _ in range(4)]
        for g in range(16):
            Q = [(qs[j, q, 0, 8 * g:8 * g + 8, :], qs[j, q, 1, 8 * g:8 * g + 8, :]) for q in range(4)]
            for r, (br, bi) in enumerate(_bfly_inv(Q)):
                rows[r].append(jnp.concatenate([br, bi], axis=0).astype(bf16))
        for r in range(4):
            yv[pl.ds(r, 128, stride=4), :] = jnp.dot(Fi_ref[r], jnp.concatenate(rows[r], axis=0),
                                                     preferred_element_type=f32)

    def loop(n, fn):
        def body(i, carry):
            fn(i)
            return carry
        lax.fori_loop(0, n, body, 0)

    def C_iter(po):
        for u in range(CU):
            C_pos(po * CU + u)

    def mod_main():
        for d in wmod_cps:
            d.wait()
        cf = c_ref[...].astype(f32)
        sc = (cf * jax.nn.sigmoid(cf)).astype(bf16)
        mod_s[:, 0:5 * D] = jnp.dot(sc, wmod_s[:, 0:5 * D], preferred_element_type=f32).astype(bf16).astype(f32)

    def mod_gb():
        cf = c_ref[...].astype(f32)
        sc = (cf * jax.nn.sigmoid(cf)).astype(bf16)
        mod_s[:, 5 * D:6 * D] = jnp.dot(sc, wmod_s[:, 5 * D:6 * D], preferred_element_type=f32).astype(bf16).astype(f32)

    def wait_T(j):
        chunk_copy(j, 0).wait()
        for t in range(4):
            T_tile(0, 4 * j + t)

    def first_F():
        wait_T(0)
        def body(j):
            chunk_copy(j, 1).wait()
            chunk_copy(j, 2).wait()
            F_chunk(0, j)
            pl.when(j + 1 < NC)(lambda: wait_T(j + 1))
        loop(NC, body)

    def I_loop(c):
        conv_copy(c + 1, 0).wait()
        def i_body(jo):
            for u in range(IU):
                I_chunk(c, jo * IU + u)
                for t in range(4):
                    T_tile(c + 1, (jo * IU + u) * 4 + t)
        loop(NC // IU, i_body)

    with scope("F0"):
        first_F()
        start_late()
    with scope("conv"):
        def tile_body(c):
            with scope("I"):
                I_loop(c - 1)
            with scope("wkv"):
                conv_copy(c, 1).wait()
                conv_copy(c, 2).wait()
            with scope("F"):
                def f_body(jo):
                    for u in range(FU):
                        F_chunk(c, jo * FU + u)
                loop(NC // FU, f_body)
            with scope("C"):
                loop(16 // CU, C_iter)
        loop(16 // CU, C_iter)
        def tb(c, carry):
            tile_body(c)
            return carry
        lax.fori_loop(1, NT, tb, 0)
        with scope("mod"):
            mod_main()

    def pre_gen(b, slot):
        for p in range(MB // PR):
            r0 = b * MB + p * PR
            if not isinstance(r0, int):
                r0 = pl.multiple_of(r0, PR)
            sa = mod_s[:, 0 * D:1 * D]
            ca = mod_s[:, 1 * D:2 * D]
            ga = mod_s[:, 2 * D:3 * D]
            sb = mod_s[:, 3 * D:4 * D]
            cb = mod_s[:, 4 * D:5 * D]
            x = q_s[pl.ds(r0, PR), :].astype(f32)
            y = jnp.concatenate([y_s[c, pl.ds(r0, PR), :] for c in range(NT)], axis=1)
            h = _ln(x) * (1.0 + ca) + sa
            x1 = (x + ga * (h * y)).astype(bf16)
            x1_s[slot, p * PR:(p + 1) * PR, :] = x1
            x1 = x1.astype(f32)
            h2_s[slot, p * PR:(p + 1) * PR, :] = (_ln(x1) * (1.0 + cb) + sb).astype(bf16)
            yield

    def mlp_gen(slot, first=False, tails=None):
        for n in range(F // 128):
            cs = slice(n * 128, (n + 1) * 128)
            a = h2_s[slot]
            if first and n in GW:
                with scope("wgw"):
                    for i in range(n * 128 // WP, GW[n]):
                        wg_cps[i].wait()
                        wu_cps[i].wait()
                    if n == Q1W:
                        q_copy(1).wait()
            g = jnp.dot(a, wg_s[:, cs], preferred_element_type=f32)
            yield
            u = jnp.dot(a, wu_s[:, cs], preferred_element_type=f32)
            hh_s[:, cs] = (jnp.maximum(g, 0.0) * u).astype(bf16)
            yield
        for n in range(NT):
            cs = slice(n * 128, (n + 1) * 128)
            acc = None
            if first and n in DW:
                with scope("wdw"):
                    wd_cps[DW[n] - 1].wait()
                    if n == 0:
                        gb_cp.wait()
            for kk in range(0, F // 128, KD):
                ks = slice(kk * 128, (kk + KD) * 128)
                d1 = jnp.dot(hh_s[:, ks], wd_s[ks, cs], preferred_element_type=f32)
                acc = d1 if acc is None else acc + d1
                if first and n == 0 and kk == 0:
                    mod_gb()
                if kk + KD >= F // 128:
                    gb = mod_s[:, 5 * D + n * 128:5 * D + (n + 1) * 128]
                    o_s[slot, :, cs] = (x1_s[slot, :, cs].astype(f32) + gb * acc).astype(bf16)
                    if tails is not None:
                        tails[n].start()
                yield
    NM = 2 * (F // 128) + NT * (F // 128 // KD)

    def out_copy(b, slot):
        return pltpu.make_async_copy(o_s.at[slot], o_hbm.at[pl.ds(pl.multiple_of(b * MB, MB), MB), :], osems.at[slot])

    def i_gen(c, chunks):
        for j in chunks:
            I_chunk(c, j)
            yield

    with scope("pre0"):
        I_chunk(NT - 1, 0)
        q_copy(0).wait()
        for _ in pre_gen(0, 0):
            pass
    with scope("blk0"):
        interleave(mlp_gen(0, first=True), NM, [(i_gen(NT - 1, range(1, NC)), NC - 1, IA, IB),
                                                (pre_gen(1, 1), MB // PR, PA, 0.95)])
        out_copy(0, 0).start()

    with scope("main"):
        def main_body(b, carry):
            slot = b % 2
            @pl.when(b >= 2)
            def _():
                out_copy(b - 2, slot).wait()
            q_copy(b + 1).wait()
            interleave(mlp_gen(slot), NM, [(pre_gen(b + 1, 1 - slot), MB // PR, 0.08, 0.9)])
            out_copy(b, slot).start()
            return carry
        lax.fori_loop(1, NB - 1, main_body, 0)
    with scope("last"):
        lb, lp = NB - 1, (NB - 1) % 2
        out_copy(NB - 3, (NB - 3) % 2).wait()
        tails = [pltpu.make_async_copy(o_s.at[lp, :, n * 128:(n + 1) * 128],
                                       o_hbm.at[lb * MB:(lb + 1) * MB, n * 128:(n + 1) * 128], osems.at[2 + n])
                 for n in range(NT)]
        for _ in mlp_gen(lp, tails=tails):
            pass
    with scope("tail"):
        out_copy(NB - 2, (NB - 2) % 2).wait()
        for d in tails:
            d.wait()


@jax.jit
def pallas_adaLN_cond__ssm_conv_h3__glu_gated_reglu__prompt_kernel(
        A_q, A_k, A_v, A_shift_k, A_ssm_k, A_ssm_D, B_x, B_W_gate, B_W_up, B_W_down, c, w_mod):
    ph = 2.0 * np.pi * (np.arange(128)[:, None] + 0.25) / 128 * np.arange(128)[None, :]
    F0 = jnp.asarray(np.concatenate([np.cos(ph), np.sin(ph)], axis=0).astype(np.float32))
    hbm = pl.BlockSpec(memory_space=pl.ANY)
    out = pl.pallas_call(
        kernel,
        out_shape=jax.ShapeDtypeStruct((S, D), A_q.dtype),
        in_specs=[hbm] * 12,
        out_specs=hbm,
        scratch_shapes=[
            pltpu.VMEM((4, D), bf16),
            pltpu.VMEM((D,), bf16),
            pltpu.VMEM((1, D), bf16),
            pltpu.VMEM((256, 128), f32),
            pltpu.VMEM((4, 256, 128), bf16),
            pltpu.VMEM((4, 128, 256), bf16),
            pltpu.VMEM((1, D), f32),
            pltpu.VMEM((NT, S + 16, 128), bf16),
            pltpu.VMEM((NT, S, 128), bf16),
            pltpu.VMEM((NT, 128, S), bf16),
            pltpu.VMEM((S, 128), bf16),
            pltpu.VMEM((NC, 4, 3, 128 + PAD, 128), f32),
            pltpu.VMEM((NC, 4, 3, 128 + PAD, 128), f32),
            pltpu.VMEM((NC, 4, 2, 128 + PAD, 128), f32),
            pltpu.VMEM((NT, S + PAD, 128), f32),
            pltpu.VMEM((S, D), bf16),
            pltpu.VMEM((D, F), bf16),
            pltpu.VMEM((D, F), bf16),
            pltpu.VMEM((F, D), bf16),
            pltpu.VMEM((D, 6 * D), bf16),
            pltpu.VMEM((1, 6 * D), f32),
            pltpu.VMEM((2, MB, D), bf16),
            pltpu.VMEM((2, MB, D), bf16),
            pltpu.VMEM((MB, F), bf16),
            pltpu.VMEM((2, MB, D), bf16),
            pltpu.SemaphoreType.DMA((3 * NT + NB + 5 + 2 * (F // WP) + NT + len(DP) - 1 + 3 * NC,)),
            pltpu.SemaphoreType.DMA((2 + NT,)),
        ],
        compiler_params=pltpu.CompilerParams(vmem_limit_bytes=120 * 1024 * 1024),
    )(A_q.reshape(S, D), A_k.reshape(S, D), A_v.reshape(S, D), A_shift_k.T, A_ssm_k, A_ssm_D,
      B_W_gate, B_W_up, B_W_down, c, w_mod, F0)
    return out.reshape(A_q.shape)
```

```python
import numpy as np
import jax
import jax.numpy as jnp
from jax import lax
import jax.experimental.pallas as pl
import jax.experimental.pallas.tpu as pltpu

S, D, F = 2048, 640, 1536
L = 512
NC = S // L
NT = D // 128
MB = 256
NB = S // MB
PR = 16
KD = 4
FU = 4
IU = 4
CU = 4
GW = {0: 1, 4: 2, 8: 3}
DW = {0: 1, 2: 2}
WP = 512
DP = (0, 2, 5)
PAD = 8
Q1W, Q1S = 4, 0
IA, IB, PA = 0.0, 0.18, 0.24
IPRE = 3
SCOPES = False
f32, bf16, u32 = jnp.float32, jnp.bfloat16, jnp.uint32


def _ln(x):
    m = jnp.sum(x, axis=-1, keepdims=True) * (1.0 / D)
    xc = x - m
    v = jnp.sum(xc * xc, axis=-1, keepdims=True) * (1.0 / D)
    return xc * lax.rsqrt(v + 1e-5)


def _lo(w):
    return lax.bitcast_convert_type(w << 16, f32)


def _hi(w):
    return lax.bitcast_convert_type(w & jnp.uint32(0xFFFF0000), f32)


def _bfly_fwd(a):
    (a0r, a0i), (a1r, a1i), (a2r, a2i), (a3r, a3i) = a
    t0r, t0i, t1r, t1i = a0r + a2r, a0i + a2i, a0r - a2r, a0i - a2i
    t2r, t2i, t3r, t3i = a1r + a3r, a1i + a3i, a1r - a3r, a1i - a3i
    return [(t0r + t2r, t0i + t2i), (t1r - t3i, t1i + t3r), (t0r - t2r, t0i - t2i), (t1r + t3i, t1i - t3r)]


def _bfly_inv(q):
    (q0r, q0i), (q1r, q1i), (q2r, q2i), (q3r, q3i) = q
    u0r, u0i, u1r, u1i = q0r + q2r, q0i + q2i, q0r - q2r, q0i - q2i
    u2r, u2i, u3r, u3i = q1r + q3r, q1i + q3i, q1r - q3r, q1i - q3i
    return [(u0r + u2r, u0i + u2i), (u1r + u3i, u1i - u3r), (u0r - u2r, u0i - u2i), (u1r - u3i, u1i + u3r)]


def interleave(main, nmain, sides):
    done = [0] * len(sides)
    i = 0
    for _ in main:
        i += 1
        f = i / nmain
        for s, (g, n, a, b) in enumerate(sides):
            want = min(n, max(0, int(np.ceil((f - a) / (b - a) * n - 1e-9))))
            while done[s] < want:
                next(g)
                done[s] += 1
    for s, (g, n, a, b) in enumerate(sides):
        while done[s] < n:
            next(g)
            done[s] += 1
        for _ in g:
            pass


class _NoScope:
    def __init__(self, name):
        pass

    def __enter__(self):
        return self

    def __exit__(self, *a):
        return False


def kernel(q_hbm, k_hbm, v_hbm, skt_hbm, ssmk_hbm, ssmd_hbm, wg_hbm, wu_hbm, wd_hbm, c_hbm, wmod_hbm,
           F0_hbm, o_hbm, skt_ref, ssmd_ref, c_ref, F0_ref, F_ref, Fi_ref, sd_s,
           k_s, v_s, ssmk_s, kt_s, xs, gs, qs, y_s, q_s, wg_s, wu_s, wd_s, wmod_s, mod_s,
           x1_s, h2_s, hh_s, o_s, sems, osems):
    scope = jax.named_scope if SCOPES else _NoScope

    def conv_copy(c, i):
        c0 = c * 128 if isinstance(c, int) else pl.multiple_of(c * 128, 128)
        if i == 0:
            return pltpu.make_async_copy(ssmk_hbm.at[pl.ds(c0, 128), :], ssmk_s.at[c], sems.at[c])
        if i == 1:
            return pltpu.make_async_copy(k_hbm.at[:, pl.ds(c0, 128)], k_s.at[c, pl.ds(16, S), :], sems.at[NT + c])
        return pltpu.make_async_copy(v_hbm.at[:, pl.ds(c0, 128)], v_s.at[c], sems.at[2 * NT + c])

    nsem = [3 * NT + NB]

    def cp(src, dst):
        nsem[0] += 1
        return pltpu.make_async_copy(src, dst, sems.at[nsem[0] - 1])
    wmod_cps = [cp(wmod_hbm.at[:, 0:5 * D], wmod_s.at[:, 0:5 * D])]
    gb_cp = cp(wmod_hbm.at[:, 5 * D:6 * D], wmod_s.at[:, 5 * D:6 * D])
    wg_cps = [cp(wg_hbm.at[:, n * WP:(n + 1) * WP], wg_s.at[:, n * WP:(n + 1) * WP]) for n in range(F // WP)]
    wu_cps = [cp(wu_hbm.at[:, n * WP:(n + 1) * WP], wu_s.at[:, n * WP:(n + 1) * WP]) for n in range(F // WP)]
    wd_cps = [cp(wd_hbm.at[:, a * 128:b * 128], wd_s.at[:, a * 128:b * 128]) for a, b in zip(DP[:-1], DP[1:])]

    def q_copy(b):
        r0 = b * MB if isinstance(b, int) else pl.multiple_of(b * MB, MB)
        return pltpu.make_async_copy(q_hbm.at[pl.ds(r0, MB), :], q_s.at[pl.ds(r0, MB), :], sems.at[3 * NT + b])

    F0_cp = cp(F0_hbm, F0_ref)
    F0_cp.start()
    small_cps = [cp(skt_hbm, skt_ref), cp(ssmd_hbm, ssmd_ref), cp(c_hbm, c_ref)]
    for d in small_cps:
        d.start()
    base0 = nsem[0]
    nsem[0] += 3 * NC

    def chunk_copy(j, i):
        r0 = j * L if isinstance(j, int) else pl.multiple_of(j * L, L)
        r16 = 16 + r0 if isinstance(j, int) else pl.multiple_of(16 + r0, 16)
        sem = sems.at[base0 + i * NC + j]
        if i == 0:
            return pltpu.make_async_copy(ssmk_hbm.at[0:128, pl.ds(r0, L)], ssmk_s.at[0, :, pl.ds(r0, L)], sem)
        if i == 1:
            return pltpu.make_async_copy(k_hbm.at[pl.ds(r0, L), 0:128], k_s.at[0, pl.ds(r16, L), :], sem)
        return pltpu.make_async_copy(v_hbm.at[pl.ds(r0, L), 0:128], v_s.at[0, pl.ds(r0, L), :], sem)
    for j in range(NC):
        chunk_copy(j, 0).start()
        chunk_copy(j, 1).start()
        chunk_copy(j, 2).start()
    for c in range(1, NT):
        for i in range(3):
            conv_copy(c, i).start()

    def start_late():
        for d in wmod_cps:
            d.start()
        q_copy(0).start()
        for n in range(F // WP):
            wg_cps[n].start()
            wu_cps[n].start()
            if n == Q1S:
                q_copy(1).start()
        gb_cp.start()
        for d in wd_cps:
            d.start()
        for b in range(2, NB):
            q_copy(b).start()

    ki = lax.broadcasted_iota(jnp.int32, (128, 128), 0)
    ang = (4 * ki + 1).astype(f32) * (2.0 * np.pi / (4 * L))
    twr, twi = jnp.cos(ang), jnp.sin(ang)
    F0_cp.wait()
    co, si = F0_ref[0:128], F0_ref[128:256]
    for r in range(4):
        if r > 0:
            co, si = co * twr - si * twi, co * twi + si * twr
        fr = jnp.concatenate([t[8 * g:8 * g + 8] for g in range(16) for t in (co, si)], axis=0)
        F_ref[r] = fr.astype(bf16)
        Fi_ref[r] = (fr * (1.0 / L)).astype(bf16).T

    for d in small_cps:
        d.wait()
    sd_s[...] = ssmd_ref[...].astype(f32).reshape(1, D)
    for c in range(NT):
        k_s[c, 0:16, :] = jnp.zeros((16, 128), bf16)

    def T_tile(c, t):
        t0 = t * 128 if isinstance(t, int) else pl.multiple_of(t * 128, 128)
        kt_s[pl.ds(t0, 128), :] = ssmk_s[c, :, pl.ds(t0, 128)].T

    def phases(wref, off):
        a = wref[pl.ds(off, 128, stride=2), :]
        b = wref[pl.ds(off + 1, 128, stride=2), :]
        return [_lo(a), _hi(a), _lo(b), _hi(b)]

    def spectrum(parts, dst, j, first, extra=None):
        for g in range(16):
            a = [(parts[r][16 * g:16 * g + 8], parts[r][16 * g + 8:16 * g + 16]) for r in range(4)]
            if extra is not None:
                a[0] = (a[0][0] + extra, a[0][1])
            for q, (re, im) in enumerate(_bfly_fwd(a)):
                if first:
                    trip = (re + im, re, im)
                else:
                    trip = (re, im - re, re + im)
                for u in range(3):
                    dst[j, q, u, 8 * g:8 * g + 8, :] = trip[u]

    def F_chunk(c, j):
        c0 = pl.multiple_of(c * 128, 128) if not isinstance(c, int) else c * 128
        w0 = j * (L // 2) if isinstance(j, int) else pl.multiple_of(j * (L // 2), L // 2)
        kk = phases(kt_s.bitcast(u32).at[pl.ds(w0, L // 2), :], 0)
        kparts = [jnp.dot(F_ref[r], kk[r].astype(bf16), preferred_element_type=f32) for r in range(4)]
        w = skt_ref[:, pl.ds(c0, 128)].astype(f32)
        kw = k_s.bitcast(u32).at[c, pl.ds(w0, L // 2 + 8), :]
        vw = v_s.bitcast(u32).at[c, pl.ds(w0, L // 2), :]
        kc = phases(kw, 8)
        kp = phases(kw, 6)
        vv = phases(vw, 0)
        taps = [[kc[0], kp[3], kp[2], kp[1]], [kc[1], kc[0], kp[3], kp[2]],
                [kc[2], kc[1], kc[0], kp[3]], [kc[3], kc[2], kc[1], kc[0]]]
        parts = []
        for r in range(4):
            ks = taps[r][0] * w[0:1] + taps[r][1] * w[1:2] + taps[r][2] * w[2:3] + taps[r][3] * w[3:4]
            kv = (ks * vv[r]).astype(bf16)
            parts.append(jnp.dot(F_ref[r], kv, preferred_element_type=f32))
        sd = jnp.where(j == 0, sd_s[:, pl.ds(c0, 128)], 0.0)
        spectrum(kparts, gs, j, False, extra=sd)
        spectrum(parts, xs, j, True)

    def C_pos(p):
        r0 = pl.multiple_of(p * 8, 8)
        for q in range(4):
            X = [tuple(xs[j, q, u, pl.ds(r0, 8), :] for u in range(3)) for j in range(NC)]
            G = [tuple(gs[m, q, u, pl.ds(r0, 8), :] for u in range(3)) for m in range(NC)]
            prev = None
            for i in range(NC):
                acc = None
                for j in range(i + 1):
                    s, xr, xi = X[j]
                    gr, d, t = G[i - j]
                    q3 = (gr * s, xr * d, xi * t)
                    acc = q3 if acc is None else (acc[0] + q3[0], acc[1] + q3[1], acc[2] + q3[2])
                pr, pi = acc[0] - acc[2], acc[0] + acc[1]
                qr, qi = (pr, pi) if prev is None else (pr + prev[1], pi - prev[0])
                prev = (pr, pi)
                qs[i, q, 0, pl.ds(r0, 8), :] = qr
                qs[i, q, 1, pl.ds(r0, 8), :] = qi

    def I_chunk(c, j):
        r0 = j * L if isinstance(j, int) else pl.multiple_of(j * L, L)
        yv = y_s.at[c, pl.ds(r0, L), :]
        rows = [[] for _ in range(4)]
        for g in range(16):
            Q = [(qs[j, q, 0, 8 * g:8 * g + 8, :], qs[j, q, 1, 8 * g:8 * g + 8, :]) for q in range(4)]
            for r, (br, bi) in enumerate(_bfly_inv(Q)):
                rows[r].append(jnp.concatenate([br, bi], axis=0).astype(bf16))
        for r in range(4):
            yv[pl.ds(r, 128, stride=4), :] = jnp.dot(Fi_ref[r], jnp.concatenate(rows[r], axis=0),
                                                     preferred_element_type=f32)

    def loop(n, fn):
        def body(i, carry):
            fn(i)
            return carry
        lax.fori_loop(0, n, body, 0)

    def C_iter(po):
        for u in range(CU):
            C_pos(po * CU + u)

    def mod_main():
        for d in wmod_cps:
            d.wait()
        cf = c_ref[...].astype(f32)
        sc = (cf * jax.nn.sigmoid(cf)).astype(bf16)
        mod_s[:, 0:5 * D] = jnp.dot(sc, wmod_s[:, 0:5 * D], preferred_element_type=f32).astype(bf16).astype(f32)

    def mod_gb():
        cf = c_ref[...].astype(f32)
        sc = (cf * jax.nn.sigmoid(cf)).astype(bf16)
        mod_s[:, 5 * D:6 * D] = jnp.dot(sc, wmod_s[:, 5 * D:6 * D], preferred_element_type=f32).astype(bf16).astype(f32)

    def wait_T(j):
        chunk_copy(j, 0).wait()
        for t in range(4):
            T_tile(0, 4 * j + t)

    def first_F():
        wait_T(0)
        def body(j):
            chunk_copy(j, 1).wait()
            chunk_copy(j, 2).wait()
            F_chunk(0, j)
            pl.when(j + 1 < NC)(lambda: wait_T(j + 1))
        loop(NC, body)

    def I_loop(c):
        conv_copy(c + 1, 0).wait()
        def i_body(jo):
            for u in range(IU):
                I_chunk(c, jo * IU + u)
                for t in range(4):
                    T_tile(c + 1, (jo * IU + u) * 4 + t)
        loop(NC // IU, i_body)

    with scope("F0"):
        first_F()
        start_late()
    with scope("conv"):
        def tile_body(c):
            with scope("I"):
                I_loop(c - 1)
            with scope("wkv"):
                conv_copy(c, 1).wait()
                conv_copy(c, 2).wait()
            with scope("F"):
                def f_body(jo):
                    for u in range(FU):
                        F_chunk(c, jo * FU + u)
                loop(NC // FU, f_body)
            with scope("C"):
                loop(16 // CU, C_iter)
        loop(16 // CU, C_iter)
        def tb(c, carry):
            tile_body(c)
            return carry
        lax.fori_loop(1, NT, tb, 0)
        for j in range(IPRE):
            I_chunk(NT - 1, j)
        with scope("mod"):
            mod_main()

    def pre_gen(b, slot):
        for p in range(MB // PR):
            r0 = b * MB + p * PR
            if not isinstance(r0, int):
                r0 = pl.multiple_of(r0, PR)
            sa = mod_s[:, 0 * D:1 * D]
            ca = mod_s[:, 1 * D:2 * D]
            ga = mod_s[:, 2 * D:3 * D]
            sb = mod_s[:, 3 * D:4 * D]
            cb = mod_s[:, 4 * D:5 * D]
            x = q_s[pl.ds(r0, PR), :].astype(f32)
            y = jnp.concatenate([y_s[c, pl.ds(r0, PR), :] for c in range(NT)], axis=1)
            h = _ln(x) * (1.0 + ca) + sa
            x1 = (x + ga * (h * y)).astype(bf16)
            x1_s[slot, p * PR:(p + 1) * PR, :] = x1
            x1 = x1.astype(f32)
            h2_s[slot, p * PR:(p + 1) * PR, :] = (_ln(x1) * (1.0 + cb) + sb).astype(bf16)
            yield

    def mlp_gen(slot, first=False, tails=None):
        for n in range(F // 128):
            cs = slice(n * 128, (n + 1) * 128)
            a = h2_s[slot]
            if first and n in GW:
                with scope("wgw"):
                    for i in range(n * 128 // WP, GW[n]):
                        wg_cps[i].wait()
                        wu_cps[i].wait()
                    if n == Q1W:
                        q_copy(1).wait()
            g = jnp.dot(a, wg_s[:, cs], preferred_element_type=f32)
            yield
            u = jnp.dot(a, wu_s[:, cs], preferred_element_type=f32)
            hh_s[:, cs] = (jnp.maximum(g, 0.0) * u).astype(bf16)
            yield
        for n in range(NT):
            cs = slice(n * 128, (n + 1) * 128)
            acc = None
            if first and n in DW:
                with scope("wdw"):
                    wd_cps[DW[n] - 1].wait()
                    if n == 0:
                        gb_cp.wait()
            for kk in range(0, F // 128, KD):
                ks = slice(kk * 128, (kk + KD) * 128)
                d1 = jnp.dot(hh_s[:, ks], wd_s[ks, cs], preferred_element_type=f32)
                acc = d1 if acc is None else acc + d1
                if first and n == 0 and kk == 0:
                    mod_gb()
                if kk + KD >= F // 128:
                    gb = mod_s[:, 5 * D + n * 128:5 * D + (n + 1) * 128]
                    o_s[slot, :, cs] = (x1_s[slot, :, cs].astype(f32) + gb * acc).astype(bf16)
                    if tails is not None:
                        tails[n].start()
                yield
    NM = 2 * (F // 128) + NT * (F // 128 // KD)

    def out_copy(b, slot):
        return pltpu.make_async_copy(o_s.at[slot], o_hbm.at[pl.ds(pl.multiple_of(b * MB, MB), MB), :], osems.at[slot])

    def i_gen(c, chunks):
        for j in chunks:
            I_chunk(c, j)
            yield

    with scope("pre0"):
        if IPRE == 0:
            I_chunk(NT - 1, 0)
        q_copy(0).wait()
        for _ in pre_gen(0, 0):
            pass
    with scope("blk0"):
        interleave(mlp_gen(0, first=True), NM, [(i_gen(NT - 1, range(max(IPRE, 1), NC)), NC - max(IPRE, 1), IA, IB),
                                                (pre_gen(1, 1), MB // PR, PA, 0.95)])
        out_copy(0, 0).start()

    with scope("main"):
        def main_body(b, carry):
            slot = b % 2
            @pl.when(b >= 2)
            def _():
                out_copy(b - 2, slot).wait()
            q_copy(b + 1).wait()
            interleave(mlp_gen(slot), NM, [(pre_gen(b + 1, 1 - slot), MB // PR, 0.08, 0.9)])
            out_copy(b, slot).start()
            return carry
        lax.fori_loop(1, NB - 1, main_body, 0)
    with scope("last"):
        lb, lp = NB - 1, (NB - 1) % 2
        out_copy(NB - 3, (NB - 3) % 2).wait()
        tails = [pltpu.make_async_copy(o_s.at[lp, :, n * 128:(n + 1) * 128],
                                       o_hbm.at[lb * MB:(lb + 1) * MB, n * 128:(n + 1) * 128], osems.at[2 + n])
                 for n in range(NT)]
        for _ in mlp_gen(lp, tails=tails):
            pass
    with scope("tail"):
        out_copy(NB - 2, (NB - 2) % 2).wait()
        for d in tails:
            d.wait()


@jax.jit
def pallas_adaLN_cond__ssm_conv_h3__glu_gated_reglu__prompt_kernel(
        A_q, A_k, A_v, A_shift_k, A_ssm_k, A_ssm_D, B_x, B_W_gate, B_W_up, B_W_down, c, w_mod):
    ph = 2.0 * np.pi * (np.arange(128)[:, None] + 0.25) / 128 * np.arange(128)[None, :]
    F0 = jnp.asarray(np.concatenate([np.cos(ph), np.sin(ph)], axis=0).astype(np.float32))
    hbm = pl.BlockSpec(memory_space=pl.ANY)
    out = pl.pallas_call(
        kernel,
        out_shape=jax.ShapeDtypeStruct((S, D), A_q.dtype),
        in_specs=[hbm] * 12,
        out_specs=hbm,
        scratch_shapes=[
            pltpu.VMEM((4, D), bf16),
            pltpu.VMEM((D,), bf16),
            pltpu.VMEM((1, D), bf16),
            pltpu.VMEM((256, 128), f32),
            pltpu.VMEM((4, 256, 128), bf16),
            pltpu.VMEM((4, 128, 256), bf16),
            pltpu.VMEM((1, D), f32),
            pltpu.VMEM((NT, S + 16, 128), bf16),
            pltpu.VMEM((NT, S, 128), bf16),
            pltpu.VMEM((NT, 128, S), bf16),
            pltpu.VMEM((S, 128), bf16),
            pltpu.VMEM((NC, 4, 3, 128 + PAD, 128), f32),
            pltpu.VMEM((NC, 4, 3, 128 + PAD, 128), f32),
            pltpu.VMEM((NC, 4, 2, 128 + PAD, 128), f32),
            pltpu.VMEM((NT, S + PAD, 128), f32),
            pltpu.VMEM((S, D), bf16),
            pltpu.VMEM((D, F), bf16),
            pltpu.VMEM((D, F), bf16),
            pltpu.VMEM((F, D), bf16),
            pltpu.VMEM((D, 6 * D), bf16),
            pltpu.VMEM((1, 6 * D), f32),
            pltpu.VMEM((2, MB, D), bf16),
            pltpu.VMEM((2, MB, D), bf16),
            pltpu.VMEM((MB, F), bf16),
            pltpu.VMEM((2, MB, D), bf16),
            pltpu.SemaphoreType.DMA((3 * NT + NB + 5 + 2 * (F // WP) + 1 + len(DP) - 1 + 3 * NC,)),
            pltpu.SemaphoreType.DMA((2 + NT,)),
        ],
        compiler_params=pltpu.CompilerParams(vmem_limit_bytes=120 * 1024 * 1024),
    )(A_q.reshape(S, D), A_k.reshape(S, D), A_v.reshape(S, D), A_shift_k.T, A_ssm_k, A_ssm_D,
      B_W_gate, B_W_up, B_W_down, c, w_mod, F0)
    return out.reshape(A_q.shape)
```
